```python
import jax
import jax.numpy as jnp

def _softmax(x, axis=-1):
    return jax.nn.softmax(x, axis=axis)

def _gelu(x):
    return jax.nn.gelu(x, approximate=True)

def _silu(x):
    return jax.nn.silu(x)

def _sigmoid(x):
    return jax.nn.sigmoid(x)

def _layernorm(x, axis=-1, eps=1e-05):
    m = jnp.mean(x, axis=axis, keepdims=True)
    v = jnp.var(x, axis=axis, keepdims=True)
    return (x - m) / jnp.sqrt(v + eps)

def _scatter_add(tgt, idx, src, axis=0):
    return tgt.at[idx].add(src)

def _segment_sum(src, seg, n):
    return jax.ops.segment_sum(src, seg, n)

class _Rng:

    def __init__(self, key):
        self._k = key

    def _next(self):
        self._k, sub = jax.random.split(self._k)
        return sub

    def normal(self, shape):
        return jax.random.normal(self._next(), shape, dtype=jnp.bfloat16)

    def randint(self, lo, hi, shape):
        return jax.random.randint(self._next(), shape, lo, hi, dtype=jnp.int32)

    def uniform(self, shape, lo=0.0, hi=1.0):
        return jax.random.uniform(self._next(), shape, jnp.bfloat16, lo, hi)

    def permutation(self, n):
        return jax.random.permutation(self._next(), n)
kernel_name = 'interleave_layers__linear_kernel_hedgehog__mixer_gmlp__prompt'

def _fwd_setup_inputs():
    _rng = _Rng(jax.random.key(int.from_bytes(__import__("os").urandom(4), "little")))
    _w = lambda a: (lambda t: t.astype(jnp.bfloat16) if jnp.issubdtype(t.dtype, jnp.floating) else t)(jnp.asarray(a))

    def _A_setup():
        B, S, D, H = (1, 2048, 640, 32)
        Dh = D // H
        return {'x': _w((lambda *s: _rng.normal(s) * 0.05)(B, S, D)), 'wqkv': _w((lambda *s: _rng.normal(s) * 0.05)(D, 3 * D)), 'w_phi': _w((lambda *s: _rng.normal(s) * 0.05)(H, Dh, Dh) * Dh ** (-0.5)), 'wo': _w((lambda *s: _rng.normal(s) * 0.05)(D, D))}
    _A_in = _A_setup()

    def _B_setup():
        B, S, D, F = (1, 2048, 640, 1536)
        Fh = F // 2
        return {'x': _w((lambda *s: _rng.normal(s) * 0.05)(B, S, D)), 'w_in': _w((lambda *s: _rng.normal(s) * 0.05)(D, 2 * Fh)), 'w_sp': _w(0.01 * (lambda *s: _rng.normal(s) * 0.05)(S, S)), 'b_sp': _w(1.0 + 0.01 * (lambda *s: _rng.normal(s) * 0.05)(S)), 'w_out': _w((lambda *s: _rng.normal(s) * 0.05)(Fh, D))}
    _B_in = _B_setup()
    return {'A_x': _A_in['x'], 'A_wqkv': _A_in['wqkv'], 'A_w_phi': _A_in['w_phi'], 'A_wo': _A_in['wo'], 'B_x': _B_in['x'], 'B_w_in': _B_in['w_in'], 'B_w_sp': _B_in['w_sp'], 'B_b_sp': _B_in['b_sp'], 'B_w_out': _B_in['w_out']}

def _fwd_reference(A_x, A_wqkv, A_w_phi, A_wo, B_x, B_w_in, B_w_sp, B_b_sp, B_w_out):

    def _A_ref(x, wqkv, w_phi, wo):
        B, S, D = x.shape
        H = 32
        Dh = D // H
        qkv = (lambda x, *d: x.transpose(*d))((x @ wqkv).reshape(B, S, 3, H, Dh), 2, 0, 3, 1, 4)
        q, k, v = (qkv[0], qkv[1], qkv[2])
        pq = jnp.einsum('bhsd,hdf->bhsf', q, w_phi)
        pk = jnp.einsum('bhsd,hdf->bhsf', k, w_phi)
        phi_q = jnp.concatenate([_softmax(pq, axis=-1), _softmax(-pq, axis=-1)], axis=-1)
        phi_k = jnp.concatenate([_softmax(pk, axis=-1), _softmax(-pk, axis=-1)], axis=-1)
        kv = jnp.einsum('bhsf,bhsd->bhfd', phi_k, v)
        z = jnp.einsum('bhsf->bhf', phi_k)
        num = jnp.einsum('bhqf,bhfd->bhqd', phi_q, kv)
        den = jnp.einsum('bhqf,bhf->bhq', phi_q, z)[..., None] + 1e-06
        o = num / den
        return (lambda x, *d: x.transpose(*d))(o, 0, 2, 1, 3).reshape(B, S, D) @ wo

    def _B_ref(x, w_in, w_sp, b_sp, w_out):
        B, S, D = x.shape
        F = w_in.shape[-1]
        Fh = F // 2
        z = _gelu(jnp.einsum('bsd,df->bsf', x, w_in))
        z1 = z[..., :Fh].copy()
        z2 = _layernorm(z[..., Fh:], axis=-1)
        g = jnp.einsum('ts,bsf->btf', w_sp, z2) + b_sp[None, :, None]
        return jnp.einsum('bsf,fd->bsd', z1 * g, w_out)
    x = A_x
    x = x + _A_ref(_layernorm(x, axis=-1), A_wqkv, A_w_phi, A_wo)
    x = x + _B_ref(_layernorm(x, axis=-1), B_w_in, B_w_sp, B_b_sp, B_w_out)
    x = x + _A_ref(_layernorm(x, axis=-1), A_wqkv, A_w_phi, A_wo)
    x = x + _B_ref(_layernorm(x, axis=-1), B_w_in, B_w_sp, B_b_sp, B_w_out)
    return x

def setup_inputs():
    _inp = _fwd_setup_inputs()
    _gk = jax.random.fold_in(jax.random.key(int.from_bytes(__import__("os").urandom(4), "little")), 2 ** 31 - 1)
    _shapes = [[1, 2048, 640]]
    _dtypes = ['bfloat16']
    _gks = jax.random.split(_gk, len(_shapes))
    _gs = [jax.random.normal(k, s, dtype=jnp.dtype(d)) * 0.05 for k, s, d in zip(_gks, _shapes, _dtypes)]
    _inp['grad_out'] = _gs[0]
    return _inp

def reference(A_x, A_wqkv, A_w_phi, A_wo, B_w_in, B_w_sp, B_b_sp, B_w_out, B_x, grad_out):
    _const = dict(B_x=B_x)

    def _f(*_d):
        return _fwd_reference(**{'A_x': _d[0], 'A_wqkv': _d[1], 'A_w_phi': _d[2], 'A_wo': _d[3], 'B_w_in': _d[4], 'B_w_sp': _d[5], 'B_b_sp': _d[6], 'B_w_out': _d[7], **_const})
    _out, _vjp = jax.vjp(_f, A_x, A_wqkv, A_w_phi, A_wo, B_w_in, B_w_sp, B_b_sp, B_w_out)
    _grads = _vjp(grad_out)
    _out0 = jnp.asarray(_out)
    return (_out0, *[jnp.asarray(_g) for _g in _grads])
```

```python
import jax
import jax.numpy as jnp
from jax import lax
import jax.experimental.pallas as pl
import jax.experimental.pallas.tpu as pltpu

S, D, H, DH = 2048, 640, 32, 20
F, FH = 1536, 768
NTL = D // 128
G = 16
NG = H // G
T = 256
NR = S // T
LN_EPS = 1e-5
DEN_EPS = 1e-6
GELU_C = 0.7978845608028654
GELU_A = 0.044715

f32 = jnp.float32
bf16 = jnp.bfloat16


def _dot_nn(a, b):
    return lax.dot_general(a, b, (((1,), (0,)), ((), ())), preferred_element_type=f32)


def _dot_nt(a, b):
    return lax.dot_general(a, b, (((1,), (1,)), ((), ())), preferred_element_type=f32)


def _dot_tn(a, b):
    return lax.dot_general(a, b, (((0,), (0,)), ((), ())), preferred_element_type=f32)


def _group_span(g):
    return DH * G * g, DH * G * (g + 1)


def _tile_groups(j):
    out = []
    for g in range(NG):
        s, e = _group_span(g)
        if s < 128 * (j + 1) and e > 128 * j:
            out.append(g)
    return out


def _bands():
    bands = []
    for a in range(NTL):
        ga = set(_tile_groups(a))
        bs = [b for b in range(NTL) if ga & set(_tile_groups(b))]
        rng = (min(bs), max(bs) + 1)
        if bands and tuple(bands[-1][2:]) == rng:
            bands[-1][1] = a + 1
        else:
            bands.append([a, a + 1, rng[0], rng[1]])
    return [tuple(b) for b in bands]


BANDS = _bands()


def _lane_iota():
    return lax.broadcasted_iota(jnp.int32, (1, 128), 1)


def _split(a, n=NTL, off=0):
    return [a[:, off + 128 * j: off + 128 * (j + 1)] for j in range(n)]


def _seg_reduce(tiles, op, ident):
    lane = _lane_iota()
    red = []
    for g in range(NG):
        s, e = _group_span(g)
        acc = None
        for j in range(NTL):
            if g not in _tile_groups(j):
                continue
            lo = max(0, s - 128 * j)
            hi = min(128, e - 128 * j)
            t = tiles[j]
            if lo > 0 or hi < 128:
                t = jnp.where((lane >= lo) & (lane < hi), t, ident)
            acc = t if acc is None else op(acc, t)
        sh = G
        while sh < 128:
            acc = op(acc, pltpu.roll(acc, sh, 1))
            sh *= 2
        red.append(acc)
    return red


def _seg_bcast(red):
    lane = _lane_iota()
    out = []
    for j in range(NTL):
        gs = _tile_groups(j)
        r = red[gs[0]]
        for g in gs[1:]:
            lo = _group_span(g)[0] - 128 * j
            r = jnp.where(lane >= lo, red[g], r)
        out.append(r)
    return out


def _head_of_lane(c):
    grp = jnp.zeros_like(c)
    for g in range(1, NG):
        grp = grp + (c >= DH * G * g).astype(jnp.int32)
    return grp * G + (c & (G - 1)), grp


def _d_of_lane(c):
    _, grp = _head_of_lane(c)
    return lax.shift_right_logical(c - grp * (DH * G), jnp.int32(G.bit_length() - 1))


def _softmax_pm(p):
    tiles = _split(p)
    mx = _seg_bcast(_seg_reduce(tiles, jnp.maximum, -jnp.inf))
    mn = _seg_bcast(_seg_reduce(tiles, jnp.minimum, jnp.inf))
    ep = [jnp.exp(t - m) for t, m in zip(tiles, mx)]
    en = [jnp.exp(m - t) for t, m in zip(tiles, mn)]
    ip = _seg_bcast([1.0 / r for r in _seg_reduce(ep, jnp.add, 0.0)])
    im = _seg_bcast([1.0 / r for r in _seg_reduce(en, jnp.add, 0.0)])
    return [e * i for e, i in zip(ep, ip)], [e * i for e, i in zip(en, im)]


def _softmax_bwd(phi_p, phi_m, dphi_p, dphi_m):
    ap = [a * b for a, b in zip(phi_p, dphi_p)]
    am = [a * b for a, b in zip(phi_m, dphi_m)]
    sp = _seg_bcast(_seg_reduce(ap, jnp.add, 0.0))
    sm = _seg_bcast(_seg_reduce(am, jnp.add, 0.0))
    return [(a - p * s) - (b - q * r)
            for a, p, s, b, q, r in zip(ap, phi_p, sp, am, phi_m, sm)]


def _ln_fwd(x):
    mu = jnp.mean(x, axis=1, keepdims=True)
    xc = x - mu
    var = jnp.mean(xc * xc, axis=1, keepdims=True)
    rstd = lax.rsqrt(var + LN_EPS)
    return xc * rstd, rstd


def _ln_bwd(dy, y, rstd):
    m1 = jnp.mean(dy, axis=1, keepdims=True)
    m2 = jnp.mean(dy * y, axis=1, keepdims=True)
    return rstd * (dy - m1 - y * m2)


def _cat(tiles):
    return jnp.concatenate(tiles, axis=1)


def _kernel(
    x_hbm, wqkv_hbm, wphi_hbm, wo_hbm, win_hbm, wsp_hbm, bsp_hbm, wout_hbm, gout_hbm,
    out_hbm, gx_hbm, gwqkv_hbm, gwphi_hbm, gwo_hbm, gwin_hbm, gwsp_hbm, gbsp_hbm, gwout_hbm,
    sA_xn, sA_pq, sA_pk, sA_v, sA_o, sB_xn, sB_z1, sB_gp, sB_g,
    x_in, gout, wqkv, mm, wo, win, wsp, bsp, wout, wcat, wop,
    xres, a_xn, a_pq, a_pk, a_v, a_o, b_xn, b_z1, b_gp, b_g,
    z2, dg, tmp, kvm, zrow, acc, dkvm, dzrow,
    d_wcat, d_wo, d_win, d_wout, stats, bcol, gphi_st, gb_st,
    in_sems, out_sems, sp_sems,
):
    in_pairs = [(x_hbm, x_in), (wqkv_hbm, wqkv), (wphi_hbm, mm), (wo_hbm, wo),
                (win_hbm, win), (wsp_hbm, wsp), (bsp_hbm, bsp), (wout_hbm, wout),
                (gout_hbm, gout)]
    in_cp = [pltpu.make_async_copy(s, d, in_sems.at[i]) for i, (s, d) in enumerate(in_pairs)]
    for c in in_cp:
        c.start()
    (IN_X, IN_WQKV, IN_WPHI, IN_WO, IN_WIN, IN_WSP, IN_BSP, IN_WOUT, IN_GOUT) = range(9)

    setA = [(a_xn, sA_xn), (a_pq, sA_pq), (a_pk, sA_pk), (a_v, sA_v), (a_o, sA_o)]
    setB = [(b_xn, sB_xn), (b_z1, sB_z1), (b_gp, sB_gp), (b_g, sB_g)]

    def spill(bufs, base, to_hbm):
        cps = []
        for i, (v, h) in enumerate(bufs):
            src, dst = (v, h) if to_hbm else (h, v)
            cps.append(pltpu.make_async_copy(src, dst, sp_sems.at[base + i]))
        return cps

    def start_all(cps):
        for c in cps:
            c.start()

    def wait_all(cps):
        for c in cps:
            c.wait()

    def rows_of(i):
        return pl.ds(pl.multiple_of(i * T, T), T)

    def row_loop(body):
        def wrapped(i, c):
            body(rows_of(i))
            return c
        lax.fori_loop(0, NR, wrapped, 0)

    def perm_matrix():
        r = lax.broadcasted_iota(jnp.int32, (D, D), 0)
        c = lax.broadcasted_iota(jnp.int32, (D, D), 1)
        hc, _ = _head_of_lane(c)
        return (r == hc * DH + _d_of_lane(c)).astype(bf16)

    def head_mask(shape, row_natural):
        r = lax.broadcasted_iota(jnp.int32, shape, 0)
        c = lax.broadcasted_iota(jnp.int32, shape, 1)
        if shape[1] > D:
            c = jnp.where(c >= D, c - D, c)
        hc, _ = _head_of_lane(c)
        if row_natural:
            return (r >= hc * DH) & (r < hc * DH + DH)
        hr, _ = _head_of_lane(r)
        return hr == hc

    in_cp[IN_WPHI].wait()
    in_cp[IN_WQKV].wait()
    mm[...] = jnp.where(head_mask((D, D), True), mm[...], jnp.zeros((), bf16))
    pm = perm_matrix()
    wcat[:, 0:D] = _dot_nn(wqkv[:, 0:D], mm[...]).astype(bf16)
    wcat[:, D:2 * D] = _dot_nn(wqkv[:, D:2 * D], mm[...]).astype(bf16)
    wcat[:, 2 * D:3 * D] = _dot_nn(wqkv[:, 2 * D:3 * D], pm).astype(bf16)
    in_cp[IN_WO].wait()
    wop[...] = _dot_tn(pm, wo[...]).astype(bf16)
    in_cp[IN_X].wait()

    d_wcat[...] = jnp.zeros_like(d_wcat)
    d_wo[...] = jnp.zeros_like(d_wo)
    d_win[...] = jnp.zeros_like(d_win)
    d_wout[...] = jnp.zeros_like(d_wout)

    def band_phi(ph, b0, b1):
        return jnp.concatenate(
            [ph[:, 128 * b0:128 * b1], ph[:, D + 128 * b0:D + 128 * b1]], axis=1)

    def band_kv(m_ref, a0, a1, b0, b1):
        return jnp.concatenate(
            [m_ref[128 * a0:128 * a1, 128 * b0:128 * b1],
             m_ref[128 * a0:128 * a1, D + 128 * b0:D + 128 * b1]], axis=1)

    def acc_bands(lhs, rhs):
        for (a0, a1, b0, b1) in BANDS:
            res = _dot_tn(lhs[:, 128 * a0:128 * a1], band_phi(rhs, b0, b1))
            nb = 128 * (b1 - b0)
            acc[128 * a0:128 * a1, 128 * b0:128 * b1] += res[:, :nb]
            acc[128 * a0:128 * a1, D + 128 * b0:D + 128 * b1] += res[:, nb:]

    def apply_nt(ph, m_ref):
        outs = []
        for (a0, a1, b0, b1) in BANDS:
            outs.append(_dot_nt(band_phi(ph, b0, b1), band_kv(m_ref, a0, a1, b0, b1)))
        return jnp.concatenate(outs, axis=1)

    def apply_nn(v, m_ref):
        plus, minus = [], []
        for (b0, b1, a0, a1) in BANDS:
            res = _dot_nn(v[:, 128 * a0:128 * a1], band_kv(m_ref, a0, a1, b0, b1))
            nb = b1 - b0
            plus += _split(res, nb)
            minus += _split(res, nb, 128 * nb)
        return plus, minus

    def a_fwd(layer):
        first = layer == 0
        slot = layer // 2
        acc[...] = jnp.zeros_like(acc)
        zrow[slot] = jnp.zeros((8, 2 * D), f32)

        def get_x(rows):
            return x_in[rows, :].astype(f32) if first else xres[rows, :]

        def phase1(rows):
            xn, rstd = _ln_fwd(get_x(rows))
            stats[rows, layer:layer + 1] = rstd
            xnb = xn.astype(bf16)
            a_xn[rows, :] = xnb
            p = _dot_nn(xnb, wcat[...])
            qp, qm = _softmax_pm(p[:, 0:D])
            a_pq[rows, :] = _cat(qp + qm).astype(bf16)
            kp, km = _softmax_pm(p[:, D:2 * D])
            phik = _cat(kp + km).astype(bf16)
            a_pk[rows, :] = phik
            vb = p[:, 2 * D:3 * D].astype(bf16)
            a_v[rows, :] = vb
            acc_bands(vb, phik)
            zrow[slot] += jnp.sum(phik.astype(f32), axis=0, keepdims=True)

        row_loop(phase1)
        kvm[slot] = jnp.where(head_mask((D, 2 * D), False), acc[...], 0.0).astype(bf16)

        def phase2(rows):
            phq = a_pq[rows, :]
            num = apply_nt(phq, kvm.at[slot])
            pz = phq.astype(f32) * zrow[slot][0:1, :]
            tl = _split(pz, 2 * NTL)
            den = _seg_reduce([a + b for a, b in zip(tl[:NTL], tl[NTL:])], jnp.add, 0.0)
            inv = _seg_bcast([1.0 / (r + DEN_EPS) for r in den])
            o = _cat([n * i for n, i in zip(_split(num), inv)]).astype(bf16)
            a_o[rows, :] = o
            xres[rows, :] = get_x(rows) + _dot_nn(o, wop[...])

        row_loop(phase2)

    def b_fwd(layer):
        slot = layer // 2
        last = layer == 3

        def phase1(rows):
            xn, rstd = _ln_fwd(xres[rows, :])
            stats[rows, layer:layer + 1] = rstd
            xnb = xn.astype(bf16)
            b_xn[rows, :] = xnb
            u = _dot_nn(xnb, win[...])
            u2 = u * u
            th = jnp.tanh(GELU_C * u * (1.0 + GELU_A * u2))
            hp = 0.5 * (1.0 + th)
            zz = u * hp
            gp = hp + (0.5 * GELU_C) * u * (1.0 - th * th) * (1.0 + 3.0 * GELU_A * u2)
            b_gp[rows, :] = gp.astype(bf16)
            b_z1[rows, :] = zz[:, :FH].astype(bf16)
            zn, rstd2 = _ln_fwd(zz[:, FH:])
            stats[rows, 4 + slot:5 + slot] = rstd2
            z2[slot, rows, :] = zn.astype(bf16)

        row_loop(phase1)

        def phase2(rows):
            g = _dot_nn(wsp[rows, :], z2[slot]) + bcol[rows, 0:1]
            b_g[rows, :] = g.astype(bf16)
            y = (b_z1[rows, :].astype(f32) * g).astype(bf16)
            xnew = xres[rows, :] + _dot_nn(y, wout[...])
            if last:
                x_in[rows, :] = xnew.astype(bf16)
            else:
                xres[rows, :] = xnew

        row_loop(phase2)

    def b_bwd(layer):
        slot = layer // 2
        first = layer == 3

        def get_d(rows):
            return gout[rows, :].astype(f32) if first else xres[rows, :]

        def phase1(rows):
            dob = get_d(rows).astype(bf16)
            dy = _dot_nt(dob, wout[...])
            z1 = b_z1[rows, :].astype(f32)
            g = b_g[rows, :].astype(f32)
            y = (z1 * g).astype(bf16)
            d_wout[...] += _dot_tn(y, dob)
            dgv = dy * z1
            dg[slot, rows, :] = dgv.astype(bf16)
            tmp[rows, :] = (dy * g * b_gp[rows, 0:FH].astype(f32)).astype(bf16)

        row_loop(phase1)

        def phase2(rows):
            dz2 = _dot_tn(wsp[:, rows], dg[slot])
            dzz = _ln_bwd(dz2, z2[slot, rows, :].astype(f32), stats[rows, 4 + slot:5 + slot])
            du2 = (dzz * b_gp[rows, FH:F].astype(f32)).astype(bf16)
            du = jnp.concatenate([tmp[rows, :], du2], axis=1)
            dxn = _dot_nt(du, win[...])
            xn = b_xn[rows, :]
            d_win[...] += _dot_tn(xn, du)
            xres[rows, :] = get_d(rows) + _ln_bwd(dxn, xn.astype(f32), stats[rows, layer:layer + 1])

        row_loop(phase2)

    def a_bwd(layer):
        slot = layer // 2
        last = layer == 0
        acc[...] = jnp.zeros_like(acc)
        dzrow[...] = jnp.zeros_like(dzrow)

        def phase1(rows):
            dob = xres[rows, :].astype(bf16)
            do = _dot_nt(dob, wop[...])
            ob = a_o[rows, :]
            d_wo[...] += _dot_tn(ob, dob)
            phq = a_pq[rows, :]
            phqf = phq.astype(f32)
            zr = zrow[slot][0:1, :]
            tl = _split(phqf * zr, 2 * NTL)
            den = _seg_reduce([a + b for a, b in zip(tl[:NTL], tl[NTL:])], jnp.add, 0.0)
            invr = [1.0 / (r + DEN_EPS) for r in den]
            inv = _seg_bcast(invr)
            dot_ = _split(do)
            dnum = _cat([a * i for a, i in zip(dot_, inv)]).astype(bf16)
            dd = _seg_reduce([a * b for a, b in zip(dot_, _split(ob.astype(f32)))], jnp.add, 0.0)
            dden = _seg_bcast([-(a * i) for a, i in zip(dd, invr)])
            acc_bands(dnum, phq)
            dp_p, dp_m = apply_nn(dnum, kvm.at[slot])
            zt = _split(zr, 2 * NTL)
            dp_p = [a + dn * z for a, dn, z in zip(dp_p, dden, zt[:NTL])]
            dp_m = [a + dn * z for a, dn, z in zip(dp_m, dden, zt[NTL:])]
            pht = _split(phqf, 2 * NTL)
            dzr = _cat([p * dn for p, dn in zip(pht, dden + dden)])
            dzrow[...] += jnp.sum(dzr, axis=0, keepdims=True)
            dpq = _softmax_bwd(pht[:NTL], pht[NTL:], dp_p, dp_m)
            tmp[rows, 0:D] = _cat(dpq).astype(bf16)

        row_loop(phase1)
        dkvm[...] = jnp.where(head_mask((D, 2 * D), False), acc[...], 0.0).astype(bf16)

        def phase2(rows):
            vb = a_v[rows, :]
            phk = a_pk[rows, :]
            dp_p, dp_m = apply_nn(vb, dkvm)
            dzt = _split(dzrow[0:1, :], 2 * NTL)
            dp_p = [a + z for a, z in zip(dp_p, dzt[:NTL])]
            dp_m = [a + z for a, z in zip(dp_m, dzt[NTL:])]
            dv = apply_nt(phk, dkvm)
            pht = _split(phk.astype(f32), 2 * NTL)
            dpk = _softmax_bwd(pht[:NTL], pht[NTL:], dp_p, dp_m)
            dP = jnp.concatenate(
                [tmp[rows, 0:D], _cat(dpk).astype(bf16), dv.astype(bf16)], axis=1)
            dxn = _dot_nt(dP, wcat[...])
            xn = a_xn[rows, :]
            d_wcat[...] += _dot_tn(xn, dP)
            dxnew = xres[rows, :] + _ln_bwd(dxn, xn.astype(f32), stats[rows, layer:layer + 1])
            if last:
                gout[rows, :] = dxnew.astype(bf16)
            else:
                xres[rows, :] = dxnew

        row_loop(phase2)

    def out_copy(i, src, dst):
        return pltpu.make_async_copy(src, dst, out_sems.at[i])

    a_fwd(0)
    spA_out = spill(setA, 0, True)
    start_all(spA_out)

    in_cp[IN_WIN].wait()
    in_cp[IN_WSP].wait()
    in_cp[IN_BSP].wait()
    in_cp[IN_WOUT].wait()
    bcol[...] = jnp.transpose(jnp.broadcast_to(bsp[...].astype(f32), (128, S)))
    b_fwd(1)
    spB_out = spill(setB, 5, True)
    start_all(spB_out)

    wait_all(spA_out)
    a_fwd(2)
    wait_all(spB_out)
    b_fwd(3)
    cp_out = out_copy(0, x_in, out_hbm)
    cp_out.start()

    in_cp[IN_GOUT].wait()
    b_bwd(3)
    spB_in = spill(setB, 5, False)
    start_all(spB_in)
    a_bwd(2)
    spA_in = spill(setA, 0, False)
    start_all(spA_in)
    wait_all(spB_in)
    b_bwd(1)

    win[...] = d_win[...].astype(bf16)
    cp_gwin = out_copy(5, win, gwin_hbm)
    cp_gwin.start()
    wout[...] = d_wout[...].astype(bf16)
    cp_gwout = out_copy(8, wout, gwout_hbm)
    cp_gwout.start()

    def wsp_grad(rows):
        wsp[rows, :] = (_dot_nt(dg[0, rows, :], z2[0]) + _dot_nt(dg[1, rows, :], z2[1])).astype(bf16)
        bcol[rows, :] = jnp.broadcast_to(
            jnp.sum(dg[0, rows, :].astype(f32) + dg[1, rows, :].astype(f32), axis=1, keepdims=True),
            (T, 128))

    row_loop(wsp_grad)
    cp_gwsp = out_copy(6, wsp, gwsp_hbm)
    cp_gwsp.start()
    gb_st[...] = jnp.transpose(bcol[...])[0:1, :].astype(bf16)
    cp_gb = out_copy(7, gb_st, gbsp_hbm)
    cp_gb.start()

    wait_all(spA_in)
    a_bwd(0)
    cp_gx = out_copy(1, gout, gx_hbm)
    cp_gx.start()

    pm = perm_matrix()
    dwq = d_wcat[:, 0:D].astype(bf16)
    dwk = d_wcat[:, D:2 * D].astype(bf16)
    dM = _dot_tn(wqkv[:, 0:D], dwq) + _dot_tn(wqkv[:, D:2 * D], dwk)
    dM = jnp.where(head_mask((D, D), True), dM, 0.0).astype(bf16)
    rr = lax.broadcasted_iota(jnp.int32, (D, 128), 0)
    rc = lax.broadcasted_iota(jnp.int32, (D, 128), 1)
    rmat = (_d_of_lane(rr) == rc).astype(bf16)
    gphi_st[...] = _dot_nn(dM, rmat)[:, 0:DH].astype(bf16)
    cp_gphi = out_copy(3, gphi_st, gwphi_hbm)
    cp_gphi.start()
    wcat[:, 0:D] = _dot_nt(dwq, mm[...]).astype(bf16)
    wcat[:, D:2 * D] = _dot_nt(dwk, mm[...]).astype(bf16)
    wcat[:, 2 * D:3 * D] = _dot_nt(d_wcat[:, 2 * D:3 * D].astype(bf16), pm).astype(bf16)
    cp_gwqkv = out_copy(2, wcat, gwqkv_hbm)
    cp_gwqkv.start()
    wo[...] = _dot_nn(pm, d_wo[...].astype(bf16)).astype(bf16)
    cp_gwo = out_copy(4, wo, gwo_hbm)
    cp_gwo.start()

    for c in (cp_out, cp_gwin, cp_gwout, cp_gwsp, cp_gb, cp_gx, cp_gphi, cp_gwqkv, cp_gwo):
        c.wait()


@jax.jit
def pallas_interleave_layers__linear_kernel_hedgehog__mixer_gmlp__prompt_kernel(
    A_x: jax.Array,
    A_wqkv: jax.Array,
    A_w_phi: jax.Array,
    A_wo: jax.Array,
    B_x: jax.Array,
    B_w_in: jax.Array,
    B_w_sp: jax.Array,
    B_b_sp: jax.Array,
    B_w_out: jax.Array,
    grad_out: jax.Array,
):
    del B_x
    x2 = A_x.reshape(S, D)
    g2 = grad_out.reshape(S, D)
    wphi_b = jnp.broadcast_to(
        A_w_phi.reshape(H * DH, 1, DH, 1), (H * DH, NG, DH, G)).reshape(D, D)
    bsp2 = B_b_sp.reshape(1, S)

    sds = jax.ShapeDtypeStruct
    out_shape = (
        sds((S, D), bf16),
        sds((S, D), bf16),
        sds((D, 3 * D), bf16),
        sds((H * DH, DH), bf16),
        sds((D, D), bf16),
        sds((D, F), bf16),
        sds((S, S), bf16),
        sds((1, S), bf16),
        sds((FH, D), bf16),
        sds((S, D), bf16), sds((S, 2 * D), bf16), sds((S, 2 * D), bf16),
        sds((S, D), bf16), sds((S, D), bf16),
        sds((S, D), bf16), sds((S, FH), bf16), sds((S, F), bf16), sds((S, FH), bf16),
    )
    any_spec = pl.BlockSpec(memory_space=pl.ANY)
    V = pltpu.VMEM
    scratch = [
        V((S, D), bf16),
        V((S, D), bf16),
        V((D, 3 * D), bf16),
        V((D, D), bf16),
        V((D, D), bf16),
        V((D, F), bf16),
        V((S, S), bf16),
        V((1, S), bf16),
        V((FH, D), bf16),
        V((D, 3 * D), bf16),
        V((D, D), bf16),
        V((S, D), f32),
        V((S, D), bf16),
        V((S, 2 * D), bf16),
        V((S, 2 * D), bf16),
        V((S, D), bf16),
        V((S, D), bf16),
        V((S, D), bf16),
        V((S, FH), bf16),
        V((S, F), bf16),
        V((S, FH), bf16),
        V((2, S, FH), bf16),
        V((2, S, FH), bf16),
        V((S, FH), bf16),
        V((2, D, 2 * D), bf16),
        V((2, 8, 2 * D), f32),
        V((D, 2 * D), f32),
        V((D, 2 * D), bf16),
        V((8, 2 * D), f32),
        V((D, 3 * D), f32),
        V((D, D), f32),
        V((D, F), f32),
        V((FH, D), f32),
        V((S, 128), f32),
        V((S, 128), f32),
        V((D, DH), bf16),
        V((1, S), bf16),
        pltpu.SemaphoreType.DMA((9,)),
        pltpu.SemaphoreType.DMA((9,)),
        pltpu.SemaphoreType.DMA((9,)),
    ]
    outs = pl.pallas_call(
        _kernel,
        out_shape=out_shape,
        in_specs=[any_spec] * 9,
        out_specs=tuple([any_spec] * len(out_shape)),
        scratch_shapes=scratch,
        compiler_params=pltpu.CompilerParams(vmem_limit_bytes=124 * 1024 * 1024),
    )(x2, A_wqkv, wphi_b, A_wo, B_w_in, B_w_sp, bsp2, B_w_out, g2)

    return (
        outs[0].reshape(1, S, D),
        outs[1].reshape(1, S, D),
        outs[2],
        outs[3].reshape(H, DH, DH),
        outs[4],
        outs[5],
        outs[6],
        outs[7].reshape(S),
        outs[8],
    )
```

```python
import jax
import jax.numpy as jnp
from jax import lax
import jax.experimental.pallas as pl
import jax.experimental.pallas.tpu as pltpu

S, D, H, DH = 2048, 640, 32, 20
F, FH = 1536, 768
NTL = D // 128
G = 8
NG = H // G
T = 512
NR = S // T
LN_EPS = 1e-5
DEN_EPS = 1e-6
GELU_C = 0.7978845608028654
GELU_A = 0.044715

f32 = jnp.float32
bf16 = jnp.bfloat16


def _dot_nn(a, b):
    return lax.dot_general(a, b, (((1,), (0,)), ((), ())), preferred_element_type=f32)


def _dot_nt(a, b):
    return lax.dot_general(a, b, (((1,), (1,)), ((), ())), preferred_element_type=f32)


def _dot_tn(a, b):
    return lax.dot_general(a, b, (((0,), (0,)), ((), ())), preferred_element_type=f32)


def _tile_groups(j):
    return [g for g in range(NG)
            if DH * G * g < 128 * (j + 1) and DH * G * (g + 1) > 128 * j]


def _bands():
    bands = []
    for a in range(NTL):
        ga = set(_tile_groups(a))
        bs = [b for b in range(NTL) if ga & set(_tile_groups(b))]
        rng = (min(bs), max(bs) + 1)
        if bands and tuple(bands[-1][2:]) == rng:
            bands[-1][1] = a + 1
        else:
            bands.append([a, a + 1, rng[0], rng[1]])
    return [tuple(b) for b in bands]


BANDS = _bands()


def _head_of_slot(c):
    grp = jnp.zeros_like(c)
    for g in range(1, NG):
        grp = grp + (c >= DH * G * g).astype(jnp.int32)
    return grp * G + (c & (G - 1)), grp


def _d_of_slot(c):
    _, grp = _head_of_slot(c)
    return lax.shift_right_logical(c - grp * (DH * G), jnp.int32(G.bit_length() - 1))


def _to4(a):
    return a.reshape(NG, DH, G, a.shape[-1])


def _from4(a):
    return a.reshape(D, a.shape[-1])


def _softmax_pm(p):
    p4 = _to4(p)
    mx = jnp.max(p4, axis=1, keepdims=True)
    mn = jnp.min(p4, axis=1, keepdims=True)
    ep = jnp.exp(p4 - mx)
    en = jnp.exp(mn - p4)
    ip = 1.0 / jnp.sum(ep, axis=1, keepdims=True)
    im = 1.0 / jnp.sum(en, axis=1, keepdims=True)
    return ep * ip, en * im


def _softmax_bwd(pp, pmn, dpp, dpm):
    ap = pp * dpp
    am = pmn * dpm
    sp = jnp.sum(ap, axis=1, keepdims=True)
    sm = jnp.sum(am, axis=1, keepdims=True)
    return (ap - pp * sp) - (am - pmn * sm)


def _ln_fwd(x):
    mu = jnp.mean(x, axis=1, keepdims=True)
    xc = x - mu
    var = jnp.mean(xc * xc, axis=1, keepdims=True)
    rstd = lax.rsqrt(var + LN_EPS)
    return xc * rstd, rstd


def _ln_bwd(dy, y, rstd):
    m1 = jnp.mean(dy, axis=1, keepdims=True)
    m2 = jnp.mean(dy * y, axis=1, keepdims=True)
    return rstd * (dy - m1 - y * m2)


def _lane_tile(col):
    return jnp.concatenate([col] * (T // 128), axis=1)


def _lane_fold(a):
    out = a[:, 0:128]
    for j in range(1, T // 128):
        out = out + a[:, 128 * j:128 * (j + 1)]
    return out


def _kernel(
    x_hbm, wqkv_hbm, wphi_hbm, wo_hbm, win_hbm, wsp_hbm, bsp_hbm, wout_hbm, gout_hbm,
    out_hbm, gx_hbm, gwqkv_hbm, gwphi_hbm, gwo_hbm, gwin_hbm, gwsp_hbm, gbsp_hbm, gwout_hbm,
    sA_xn, sA_pq, sA_pk, sA_v, sA_o, sB_xn, sB_z1, sB_gp, sB_g,
    x_in, gout, wqkv, mm, wo, win, wsp, bsp, wout, wcat, wcatT, wop,
    xres, a_xn, a_pq, a_pk, a_v, a_o, b_xn, b_z1, b_gp, b_g,
    z2, dg, tmp, tmpT, kvm, kvT, zcol, acc, dkvm, dkvT, dzcol, pmat,
    d_wcatT, d_wo, d_win, d_wout, stats, bcol, gphi_st, gb_st,
    in_sems, out_sems, sp_sems,
):
    in_pairs = [(x_hbm, x_in), (wqkv_hbm, wqkv), (wphi_hbm, mm), (wo_hbm, wo),
                (win_hbm, win), (wsp_hbm, wsp), (bsp_hbm, bsp), (wout_hbm, wout),
                (gout_hbm, gout)]
    in_cp = [pltpu.make_async_copy(s, d, in_sems.at[i]) for i, (s, d) in enumerate(in_pairs)]
    (IN_X, IN_WQKV, IN_WPHI, IN_WO, IN_WIN, IN_WSP, IN_BSP, IN_WOUT, IN_GOUT) = range(9)
    for i in (IN_WPHI, IN_WQKV, IN_X, IN_WO):
        in_cp[i].start()

    setA = [(a_xn, sA_xn), (a_pq, sA_pq), (a_pk, sA_pk), (a_v, sA_v), (a_o, sA_o)]
    setB = [(b_xn, sB_xn), (b_z1, sB_z1), (b_gp, sB_gp), (b_g, sB_g)]

    def spill(bufs, base, to_hbm):
        cps = []
        for i, (v, h) in enumerate(bufs):
            src, dst = (v, h) if to_hbm else (h, v)
            cps.append(pltpu.make_async_copy(src, dst, sp_sems.at[base + i]))
        return cps

    def start_all(cps):
        for c in cps:
            c.start()

    def wait_all(cps):
        for c in cps:
            c.wait()

    def row_loop(body, name):
        del name

        def wrapped(i, c):
            body(pl.ds(pl.multiple_of(i * T, T), T))
            return c
        lax.fori_loop(0, NR, wrapped, 0)

    def row_loop_pf(body, name):
        del name

        def wrapped(i, c):
            nxt = jnp.minimum(i + 1, NR - 1)
            body(pl.ds(pl.multiple_of(i * T, T), T), pl.ds(pl.multiple_of(nxt * T, T), T))
            return c
        lax.fori_loop(0, NR, wrapped, 0)

    def perm_matrix():
        r = lax.broadcasted_iota(jnp.int32, (D, D), 0)
        c = lax.broadcasted_iota(jnp.int32, (D, D), 1)
        hc, _ = _head_of_slot(c)
        return (r == hc * DH + _d_of_slot(c)).astype(bf16)

    def head_mask(shape, row_natural):
        r = lax.broadcasted_iota(jnp.int32, shape, 0)
        c = lax.broadcasted_iota(jnp.int32, shape, 1)
        if shape[1] > D:
            c = jnp.where(c >= D, c - D, c)
        hc, _ = _head_of_slot(c)
        if row_natural:
            return (r >= hc * DH) & (r < hc * DH + DH)
        hr, _ = _head_of_slot(r)
        return hr == hc

    d_wcatT[...] = jnp.zeros_like(d_wcatT)
    d_wo[...] = jnp.zeros_like(d_wo)
    d_win[...] = jnp.zeros_like(d_win)
    d_wout[...] = jnp.zeros_like(d_wout)
    pmat[...] = perm_matrix()
    in_cp[IN_WPHI].wait()
    in_cp[IN_WQKV].wait()
    mm[...] = jnp.where(head_mask((D, D), True), mm[...], jnp.zeros((), bf16))
    for i in (IN_WIN, IN_WSP, IN_BSP, IN_WOUT, IN_GOUT):
        in_cp[i].start()

    def band_right(lhs_ref, c0, m_ref, out_ref, outT_ref):
        for (b0, b1, a0, a1) in BANDS:
            res = _dot_nn(lhs_ref[:, c0 + 128 * a0:c0 + 128 * a1],
                          m_ref[128 * a0:128 * a1, 128 * b0:128 * b1])
            out_ref[:, c0 + 128 * b0:c0 + 128 * b1] = res.astype(bf16)
            outT_ref[c0 + 128 * b0:c0 + 128 * b1, :] = jnp.transpose(res).astype(bf16)

    band_right(wqkv, 0, mm, wcat, wcatT)
    band_right(wqkv, D, mm, wcat, wcatT)
    band_right(wqkv, 2 * D, pmat, wcat, wcatT)
    in_cp[IN_WO].wait()
    for (b0, b1, a0, a1) in BANDS:
        wop[128 * b0:128 * b1, :] = _dot_tn(
            pmat[128 * a0:128 * a1, 128 * b0:128 * b1], wo[128 * a0:128 * a1, :]).astype(bf16)
    in_cp[IN_X].wait()

    def rows_pm(ph, b0, b1):
        return jnp.concatenate(
            [ph[128 * b0:128 * b1, :], ph[D + 128 * b0:D + 128 * b1, :]], axis=0)

    def acc_bands(vT, phT):
        for (a0, a1, b0, b1) in BANDS:
            res = _dot_nt(rows_pm(phT, b0, b1), vT[128 * a0:128 * a1, :])
            nb = 128 * (b1 - b0)
            acc[128 * b0:128 * b1, 128 * a0:128 * a1] += res[:nb, :]
            acc[D + 128 * b0:D + 128 * b1, 128 * a0:128 * a1] += res[nb:, :]

    def finish_acc(m_ref, mT_ref):
        r = lax.broadcasted_iota(jnp.int32, (2 * D, D), 0)
        c = lax.broadcasted_iota(jnp.int32, (2 * D, D), 1)
        r = jnp.where(r >= D, r - D, r)
        same = _head_of_slot(r)[0] == _head_of_slot(c)[0]
        m = jnp.where(same, acc[...], 0.0)
        mT_ref[...] = m.astype(bf16)
        m_ref[...] = jnp.transpose(m).astype(bf16)

    def apply_to_v(m_ref, phT):
        outs = []
        for (a0, a1, b0, b1) in BANDS:
            lhs = jnp.concatenate(
                [m_ref[128 * a0:128 * a1, 128 * b0:128 * b1],
                 m_ref[128 * a0:128 * a1, D + 128 * b0:D + 128 * b1]], axis=1)
            outs.append(_dot_nn(lhs, rows_pm(phT, b0, b1)))
        return jnp.concatenate(outs, axis=0)

    def apply_to_phi(mT_ref, vT):
        plus, minus = [], []
        for (b0, b1, a0, a1) in BANDS:
            lhs = jnp.concatenate(
                [mT_ref[128 * b0:128 * b1, 128 * a0:128 * a1],
                 mT_ref[D + 128 * b0:D + 128 * b1, 128 * a0:128 * a1]], axis=0)
            res = _dot_nn(lhs, vT[128 * a0:128 * a1, :])
            nb = 128 * (b1 - b0)
            plus.append(res[:nb, :])
            minus.append(res[nb:, :])
        return jnp.concatenate(plus, axis=0), jnp.concatenate(minus, axis=0)

    def fold_col(ref):
        ref[...] = jnp.broadcast_to(jnp.sum(ref[...], axis=1, keepdims=True), ref.shape)

    def inv_den(phq_f, slot):
        pz = phq_f * _lane_tile(zcol[slot])
        den = (jnp.sum(_to4(pz[0:D]), axis=1, keepdims=True)
               + jnp.sum(_to4(pz[D:2 * D]), axis=1, keepdims=True))
        return 1.0 / (den + DEN_EPS)

    def a_fwd(layer):
        first = layer == 0
        slot = layer // 2
        acc[...] = jnp.zeros_like(acc)
        zcol[slot] = jnp.zeros((2 * D, 128), f32)

        def get_x(rows):
            return x_in[rows, :].astype(f32) if first else xres[rows, :]

        def ln_in(rows):
            xn, rstd = _ln_fwd(get_x(rows))
            stats[rows, layer:layer + 1] = rstd
            a_xn[rows, :] = xn.astype(bf16)

        ln_in(pl.ds(0, T))

        def phase1(rows, nrows):
            xnb = a_xn[rows, :]
            pk = _dot_nt(wcatT[D:2 * D, :], xnb)
            ln_in(nrows)
            vb = _dot_nt(wcatT[2 * D:3 * D, :], xnb).astype(bf16)
            a_v[:, rows] = vb
            kp, km = _softmax_pm(pk)
            pq = _dot_nt(wcatT[0:D, :], xnb)
            phik = jnp.concatenate([_from4(kp), _from4(km)], axis=0).astype(bf16)
            a_pk[:, rows] = phik
            acc_bands(vb, phik)
            qp, qm = _softmax_pm(pq)
            a_pq[0:D, rows] = _from4(qp).astype(bf16)
            a_pq[D:2 * D, rows] = _from4(qm).astype(bf16)
            zcol[slot] += _lane_fold(phik.astype(f32))

        row_loop_pf(phase1, "a_fwd_p1")
        finish_acc(kvm.at[slot], kvT.at[slot])
        fold_col(zcol.at[slot])

        def phase2(rows):
            phq = a_pq[:, rows]
            num = apply_to_v(kvm.at[slot], phq)
            inv = inv_den(phq.astype(f32), slot)
            o = _from4(_to4(num) * inv).astype(bf16)
            a_o[:, rows] = o
            xres[rows, :] = get_x(rows) + _dot_tn(o, wop[...])

        row_loop(phase2, "a_fwd_p2")

    def b_fwd(layer):
        slot = layer // 2
        last = layer == 3

        def ln_in(rows):
            xn, rstd = _ln_fwd(xres[rows, :])
            stats[rows, layer:layer + 1] = rstd
            b_xn[rows, :] = xn.astype(bf16)

        ln_in(pl.ds(0, T))

        def phase1(rows, nrows):
            xnb = b_xn[rows, :]

            def gelu_chunk(u, c0):
                u2 = u * u
                th = jnp.tanh(u * ((GELU_C * GELU_A) * u2 + GELU_C))
                hp = 0.5 * th + 0.5
                zz = u * hp
                gp = hp + (zz * (1.0 - hp)) * ((6.0 * GELU_C * GELU_A) * u2 + 2.0 * GELU_C)
                b_gp[rows, c0:c0 + u.shape[1]] = gp.astype(bf16)
                return zz

            ub = _dot_nn(xnb, win[:, FH:F])
            ln_in(nrows)
            ua = _dot_nn(xnb, win[:, 0:FH // 2])
            zzb = gelu_chunk(ub, FH)
            zn, rstd2 = _ln_fwd(zzb)
            stats[rows, 4 + slot:5 + slot] = rstd2
            z2[slot, rows, :] = zn.astype(bf16)
            uc = _dot_nn(xnb, win[:, FH // 2:FH])
            b_z1[rows, 0:FH // 2] = gelu_chunk(ua, 0).astype(bf16)
            b_z1[rows, FH // 2:FH] = gelu_chunk(uc, FH // 2).astype(bf16)

        row_loop_pf(phase1, "b_fwd_p1")

        def phase2(rows):
            g = _dot_nn(wsp[rows, :], z2[slot]) + bcol[rows, 0:1]
            b_g[rows, :] = g.astype(bf16)
            y = (b_z1[rows, :].astype(f32) * g).astype(bf16)
            xnew = xres[rows, :] + _dot_nn(y, wout[...])
            if last:
                x_in[rows, :] = xnew.astype(bf16)
            else:
                xres[rows, :] = xnew

        row_loop(phase2, "b_fwd_p2")

    def b_bwd(layer):
        slot = layer // 2
        first = layer == 3

        def get_d(rows):
            return gout[rows, :].astype(f32) if first else xres[rows, :]

        def phase1(rows):
            dob = get_d(rows).astype(bf16)
            dy = _dot_nt(dob, wout[...])
            z1 = b_z1[rows, :].astype(f32)
            g = b_g[rows, :].astype(f32)
            y = (z1 * g).astype(bf16)
            d_wout[...] += _dot_tn(y, dob)
            dgv = dy * z1
            dg[slot, rows, :] = dgv.astype(bf16)
            tmp[rows, :] = (dy * g * b_gp[rows, 0:FH].astype(f32)).astype(bf16)

        row_loop(phase1, "b_bwd_p1")

        def phase2(rows):
            dz2 = _dot_tn(wsp[:, rows], dg[slot])
            du1 = tmp[rows, :]
            xn = b_xn[rows, :]
            dxn1 = _dot_nt(du1, win[:, 0:FH])
            dzz = _ln_bwd(dz2, z2[slot, rows, :].astype(f32), stats[rows, 4 + slot:5 + slot])
            du2 = (dzz * b_gp[rows, FH:F].astype(f32)).astype(bf16)
            d_win[:, 0:FH] += _dot_tn(xn, du1)
            dxn = dxn1 + _dot_nt(du2, win[:, FH:F])
            d_win[:, FH:F] += _dot_tn(xn, du2)
            xres[rows, :] = get_d(rows) + _ln_bwd(dxn, xn.astype(f32), stats[rows, layer:layer + 1])

        row_loop(phase2, "b_bwd_p2")

    def a_bwd(layer):
        slot = layer // 2
        last = layer == 0
        acc[...] = jnp.zeros_like(acc)
        dzcol[...] = jnp.zeros_like(dzcol)

        def phase1(rows):
            dob = xres[rows, :].astype(bf16)
            doT = _to4(_dot_nt(wop[...], dob))
            ob = a_o[:, rows]
            d_wo[...] += _dot_nn(ob, dob)
            phq = a_pq[:, rows]
            phqf = phq.astype(f32)
            inv = inv_den(phqf, slot)
            dnum = _from4(doT * inv).astype(bf16)
            dden = -jnp.sum(doT * _to4(ob.astype(f32)), axis=1, keepdims=True) * inv
            dp_p, dp_m = apply_to_phi(kvT.at[slot], dnum)
            acc_bands(dnum, phq)
            zt = _lane_tile(zcol[slot])
            dp_p = _to4(dp_p) + dden * _to4(zt[0:D])
            dp_m = _to4(dp_m) + dden * _to4(zt[D:2 * D])
            pp = _to4(phqf[0:D])
            pmn = _to4(phqf[D:2 * D])
            dzcol[0:D, :] += _lane_fold(_from4(pp * dden))
            dzcol[D:2 * D, :] += _lane_fold(_from4(pmn * dden))
            tmpT[:, rows] = _from4(_softmax_bwd(pp, pmn, dp_p, dp_m)).astype(bf16)

        row_loop(phase1, "a_bwd_p1")
        finish_acc(dkvm, dkvT)
        fold_col(dzcol)

        def phase2(rows):
            vb = a_v[:, rows]
            phk = a_pk[:, rows]
            dp_p, dp_m = apply_to_phi(dkvT, vb)
            dv = apply_to_v(dkvm, phk)
            dzt = _lane_tile(dzcol[...])
            dp_p = _to4(dp_p + dzt[0:D])
            dp_m = _to4(dp_m + dzt[D:2 * D])
            phkf = phk.astype(f32)
            dpk = _softmax_bwd(_to4(phkf[0:D]), _to4(phkf[D:2 * D]), dp_p, dp_m)
            dPT = jnp.concatenate(
                [tmpT[:, rows], _from4(dpk).astype(bf16), dv.astype(bf16)], axis=0)
            dxn = jnp.transpose(_dot_nn(wcat[...], dPT))
            xn = a_xn[rows, :]
            d_wcatT[...] += _dot_nn(dPT, xn)
            dxnew = xres[rows, :] + _ln_bwd(dxn, xn.astype(f32), stats[rows, layer:layer + 1])
            if last:
                gout[rows, :] = dxnew.astype(bf16)
            else:
                xres[rows, :] = dxnew

        row_loop(phase2, "a_bwd_p2")

    def out_copy(i, src, dst):
        return pltpu.make_async_copy(src, dst, out_sems.at[i])

    a_fwd(0)
    spA_out = spill(setA, 0, True)
    start_all(spA_out)

    in_cp[IN_WIN].wait()
    in_cp[IN_WSP].wait()
    in_cp[IN_BSP].wait()
    in_cp[IN_WOUT].wait()
    bcol[...] = jnp.transpose(jnp.broadcast_to(bsp[...].astype(f32), (128, S)))
    b_fwd(1)
    spB_out = spill(setB, 5, True)
    start_all(spB_out)

    wait_all(spA_out)
    a_fwd(2)
    wait_all(spB_out)
    b_fwd(3)
    cp_out = out_copy(0, x_in, out_hbm)
    cp_out.start()

    in_cp[IN_GOUT].wait()
    b_bwd(3)
    spB_in = spill(setB, 5, False)
    start_all(spB_in)
    a_bwd(2)
    spA_in = spill(setA, 0, False)
    start_all(spA_in)
    wait_all(spB_in)
    b_bwd(1)

    win[...] = d_win[...].astype(bf16)
    cp_gwin = out_copy(5, win, gwin_hbm)
    cp_gwin.start()
    wout[...] = d_wout[...].astype(bf16)
    cp_gwout = out_copy(8, wout, gwout_hbm)
    cp_gwout.start()

    def wsp_grad(rows):
        wsp[rows, :] = (_dot_nt(dg[0, rows, :], z2[0]) + _dot_nt(dg[1, rows, :], z2[1])).astype(bf16)
        bcol[rows, :] = jnp.broadcast_to(
            jnp.sum(dg[0, rows, :].astype(f32) + dg[1, rows, :].astype(f32), axis=1, keepdims=True),
            (T, 128))

    row_loop(wsp_grad, "wsp_grad")
    cp_gwsp = out_copy(6, wsp, gwsp_hbm)
    cp_gwsp.start()
    gb_st[...] = jnp.transpose(bcol[...])[0:1, :].astype(bf16)
    cp_gb = out_copy(7, gb_st, gbsp_hbm)
    cp_gb.start()

    wait_all(spA_in)
    a_bwd(0)
    cp_gx = out_copy(1, gout, gx_hbm)
    cp_gx.start()

    wcatT[...] = d_wcatT[...].astype(bf16)
    rr = lax.broadcasted_iota(jnp.int32, (D, 128), 0)
    rc = lax.broadcasted_iota(jnp.int32, (D, 128), 1)
    rmat = (_d_of_slot(rr) == rc).astype(bf16)
    hm = head_mask((D, D), True)
    for (a0, a1, b0, b1) in BANDS:
        dMT = (_dot_nn(wcatT[128 * b0:128 * b1, :], wqkv[:, 128 * a0:128 * a1])
               + _dot_nn(wcatT[D + 128 * b0:D + 128 * b1, :], wqkv[:, D + 128 * a0:D + 128 * a1]))
        dM = jnp.where(hm[128 * a0:128 * a1, 128 * b0:128 * b1], jnp.transpose(dMT), 0.0)
        res = _dot_nn(dM.astype(bf16), rmat[128 * b0:128 * b1, :])
        gphi_st[128 * a0:128 * a1, :] = res[:, 0:DH].astype(bf16)
    cp_gphi = out_copy(3, gphi_st, gwphi_hbm)
    cp_gphi.start()

    for c0, m_ref in ((0, mm), (D, mm), (2 * D, pmat)):
        for (a0, a1, b0, b1) in BANDS:
            res = _dot_nn(m_ref[128 * a0:128 * a1, 128 * b0:128 * b1],
                          wcatT[c0 + 128 * b0:c0 + 128 * b1, :])
            wcat[:, c0 + 128 * a0:c0 + 128 * a1] = jnp.transpose(res).astype(bf16)
    cp_gwqkv = out_copy(2, wcat, gwqkv_hbm)
    cp_gwqkv.start()
    for (a0, a1, b0, b1) in BANDS:
        wo[128 * a0:128 * a1, :] = _dot_nn(
            pmat[128 * a0:128 * a1, 128 * b0:128 * b1],
            d_wo[128 * b0:128 * b1, :].astype(bf16)).astype(bf16)
    cp_gwo = out_copy(4, wo, gwo_hbm)
    cp_gwo.start()
    for c in (cp_out, cp_gwin, cp_gwout, cp_gwsp, cp_gb, cp_gx, cp_gphi, cp_gwqkv, cp_gwo):
        c.wait()


@jax.jit
def pallas_interleave_layers__linear_kernel_hedgehog__mixer_gmlp__prompt_kernel(
    A_x: jax.Array,
    A_wqkv: jax.Array,
    A_w_phi: jax.Array,
    A_wo: jax.Array,
    B_x: jax.Array,
    B_w_in: jax.Array,
    B_w_sp: jax.Array,
    B_b_sp: jax.Array,
    B_w_out: jax.Array,
    grad_out: jax.Array,
):
    del B_x
    x2 = A_x.reshape(S, D)
    g2 = grad_out.reshape(S, D)
    wphi_b = jnp.broadcast_to(
        A_w_phi.reshape(H * DH, 1, DH, 1), (H * DH, NG, DH, G)).reshape(D, D)
    bsp2 = B_b_sp.reshape(1, S)

    sds = jax.ShapeDtypeStruct
    out_shape = (
        sds((S, D), bf16),
        sds((S, D), bf16),
        sds((D, 3 * D), bf16),
        sds((H * DH, DH), bf16),
        sds((D, D), bf16),
        sds((D, F), bf16),
        sds((S, S), bf16),
        sds((1, S), bf16),
        sds((FH, D), bf16),
        sds((S, D), bf16), sds((2 * D, S), bf16), sds((2 * D, S), bf16),
        sds((D, S), bf16), sds((D, S), bf16),
        sds((S, D), bf16), sds((S, FH), bf16), sds((S, F), bf16), sds((S, FH), bf16),
    )
    any_spec = pl.BlockSpec(memory_space=pl.ANY)
    V = pltpu.VMEM
    scratch = [
        V((S, D), bf16),
        V((S, D), bf16),
        V((D, 3 * D), bf16),
        V((D, D), bf16),
        V((D, D), bf16),
        V((D, F), bf16),
        V((S, S), bf16),
        V((1, S), bf16),
        V((FH, D), bf16),
        V((D, 3 * D), bf16),
        V((3 * D, D), bf16),
        V((D, D), bf16),
        V((S, D), f32),
        V((S, D), bf16),
        V((2 * D, S), bf16),
        V((2 * D, S), bf16),
        V((D, S), bf16),
        V((D, S), bf16),
        V((S, D), bf16),
        V((S, FH), bf16),
        V((S, F), bf16),
        V((S, FH), bf16),
        V((2, S, FH), bf16),
        V((2, S, FH), bf16),
        V((S, FH), bf16),
        V((D, S), bf16),
        V((2, D, 2 * D), bf16),
        V((2, 2 * D, D), bf16),
        V((2, 2 * D, 128), f32),
        V((2 * D, D), f32),
        V((D, 2 * D), bf16),
        V((2 * D, D), bf16),
        V((2 * D, 128), f32),
        V((D, D), bf16),
        V((3 * D, D), f32),
        V((D, D), f32),
        V((D, F), f32),
        V((FH, D), f32),
        V((S, 128), f32),
        V((S, 128), f32),
        V((D, DH), bf16),
        V((1, S), bf16),
        pltpu.SemaphoreType.DMA((9,)),
        pltpu.SemaphoreType.DMA((9,)),
        pltpu.SemaphoreType.DMA((9,)),
    ]
    outs = pl.pallas_call(
        _kernel,
        out_shape=out_shape,
        in_specs=[any_spec] * 9,
        out_specs=tuple([any_spec] * len(out_shape)),
        scratch_shapes=scratch,
        compiler_params=pltpu.CompilerParams(vmem_limit_bytes=124 * 1024 * 1024),
    )(x2, A_wqkv, wphi_b, A_wo, B_w_in, B_w_sp, bsp2, B_w_out, g2)

    return (
        outs[0].reshape(1, S, D),
        outs[1].reshape(1, S, D),
        outs[2],
        outs[3].reshape(H, DH, DH),
        outs[4],
        outs[5],
        outs[6],
        outs[7].reshape(S),
        outs[8],
    )
```

```python
import jax
import jax.numpy as jnp
from jax import lax
import jax.experimental.pallas as pl
import jax.experimental.pallas.tpu as pltpu

S, D, H, DH = 2048, 640, 32, 20
F, FH = 1536, 768
NTL = D // 128
G = 8
NG = H // G
T = 512
NR = S // T
LN_EPS = 1e-5
DEN_EPS = 1e-6
GELU_C = 0.7978845608028654
GELU_A = 0.044715

f32 = jnp.float32
bf16 = jnp.bfloat16


def _dot_nn(a, b):
    return lax.dot_general(a, b, (((1,), (0,)), ((), ())), preferred_element_type=f32)


def _dot_nt(a, b):
    return lax.dot_general(a, b, (((1,), (1,)), ((), ())), preferred_element_type=f32)


def _dot_tn(a, b):
    return lax.dot_general(a, b, (((0,), (0,)), ((), ())), preferred_element_type=f32)


def _tile_groups(j):
    return [g for g in range(NG)
            if DH * G * g < 128 * (j + 1) and DH * G * (g + 1) > 128 * j]


def _bands():
    bands = []
    for a in range(NTL):
        ga = set(_tile_groups(a))
        bs = [b for b in range(NTL) if ga & set(_tile_groups(b))]
        rng = (min(bs), max(bs) + 1)
        if bands and tuple(bands[-1][2:]) == rng:
            bands[-1][1] = a + 1
        else:
            bands.append([a, a + 1, rng[0], rng[1]])
    return [tuple(b) for b in bands]


BANDS = _bands()


def _head_of_slot(c):
    grp = jnp.zeros_like(c)
    for g in range(1, NG):
        grp = grp + (c >= DH * G * g).astype(jnp.int32)
    return grp * G + (c & (G - 1)), grp


def _d_of_slot(c):
    _, grp = _head_of_slot(c)
    return lax.shift_right_logical(c - grp * (DH * G), jnp.int32(G.bit_length() - 1))


def _to4(a):
    return a.reshape(NG, DH, G, a.shape[-1])


def _from4(a):
    return a.reshape(D, a.shape[-1])


def _softmax_pm(p):
    p4 = _to4(p)
    mx = jnp.max(p4, axis=1, keepdims=True)
    mn = jnp.min(p4, axis=1, keepdims=True)
    ep = jnp.exp(p4 - mx)
    en = jnp.exp(mn - p4)
    ip = 1.0 / jnp.sum(ep, axis=1, keepdims=True)
    im = 1.0 / jnp.sum(en, axis=1, keepdims=True)
    return ep * ip, en * im


def _softmax_bwd(pp, pmn, dpp, dpm):
    ap = pp * dpp
    am = pmn * dpm
    sp = jnp.sum(ap, axis=1, keepdims=True)
    sm = jnp.sum(am, axis=1, keepdims=True)
    return (ap - pp * sp) - (am - pmn * sm)


def _ln_fwd(x):
    mu = jnp.mean(x, axis=1, keepdims=True)
    xc = x - mu
    var = jnp.mean(xc * xc, axis=1, keepdims=True)
    rstd = lax.rsqrt(var + LN_EPS)
    return xc * rstd, rstd


def _ln_bwd(dy, y, rstd):
    m1 = jnp.mean(dy, axis=1, keepdims=True)
    m2 = jnp.mean(dy * y, axis=1, keepdims=True)
    return rstd * (dy - m1 - y * m2)


def _lane_tile(col):
    return jnp.concatenate([col] * (T // 128), axis=1)


def _lane_fold(a):
    out = a[:, 0:128]
    for j in range(1, T // 128):
        out = out + a[:, 128 * j:128 * (j + 1)]
    return out


def _kernel(
    x_hbm, wqkv_hbm, wphi_hbm, wo_hbm, win_hbm, wsp_hbm, bsp_hbm, wout_hbm, gout_hbm,
    out_hbm, gx_hbm, gwqkv_hbm, gwphi_hbm, gwo_hbm, gwin_hbm, gwsp_hbm, gbsp_hbm, gwout_hbm,
    sA_xn, sA_pq, sA_pk, sA_v, sA_o, sB_xn, sB_z1, sB_gp, sB_g,
    x_in, gout, wqkv, mm, wo, win, wsp, bsp, wout, wcat, wcatT, wop,
    xres, a_xn, a_pq, a_pk, a_v, a_o, b_xn, b_z1, b_gp, b_g,
    z2, dg, tmp, tmpT, kvm, kvT, zcol, acc, dkvm, dkvT, dzcol, pmat,
    d_wcatT, d_wo, d_win, d_wout, stats, bcol, gphi_st, gb_st,
    in_sems, out_sems, sp_sems,
):
    in_pairs = [(x_hbm, x_in), (wqkv_hbm, wqkv), (wphi_hbm, mm), (wo_hbm, wo),
                (win_hbm, win), (wsp_hbm, wsp), (bsp_hbm, bsp), (wout_hbm, wout),
                (gout_hbm, gout)]
    in_cp = [pltpu.make_async_copy(s, d, in_sems.at[i]) for i, (s, d) in enumerate(in_pairs)]
    (IN_X, IN_WQKV, IN_WPHI, IN_WO, IN_WIN, IN_WSP, IN_BSP, IN_WOUT, IN_GOUT) = range(9)
    for i in (IN_WPHI, IN_WQKV, IN_X, IN_WO):
        in_cp[i].start()

    setA = [(a_xn, sA_xn), (a_pq, sA_pq), (a_pk, sA_pk), (a_v, sA_v), (a_o, sA_o)]
    setB = [(b_xn, sB_xn), (b_z1, sB_z1), (b_gp, sB_gp), (b_g, sB_g)]

    def spill(bufs, base, to_hbm):
        cps = []
        for i, (v, h) in enumerate(bufs):
            src, dst = (v, h) if to_hbm else (h, v)
            cps.append(pltpu.make_async_copy(src, dst, sp_sems.at[base + i]))
        return cps

    def start_all(cps):
        for c in cps:
            c.start()

    def wait_all(cps):
        for c in cps:
            c.wait()

    def row_loop(body, name):
        del name

        def wrapped(i, c):
            body(pl.ds(pl.multiple_of(i * T, T), T))
            return c
        lax.fori_loop(0, NR, wrapped, 0)

    def row_loop_pf(body, name):
        del name

        def wrapped(i, c):
            nxt = jnp.minimum(i + 1, NR - 1)
            body(pl.ds(pl.multiple_of(i * T, T), T), pl.ds(pl.multiple_of(nxt * T, T), T))
            return c
        lax.fori_loop(0, NR, wrapped, 0)

    def perm_matrix():
        r = lax.broadcasted_iota(jnp.int32, (D, D), 0)
        c = lax.broadcasted_iota(jnp.int32, (D, D), 1)
        hc, _ = _head_of_slot(c)
        return (r == hc * DH + _d_of_slot(c)).astype(bf16)

    def head_mask(shape, row_natural):
        r = lax.broadcasted_iota(jnp.int32, shape, 0)
        c = lax.broadcasted_iota(jnp.int32, shape, 1)
        if shape[1] > D:
            c = jnp.where(c >= D, c - D, c)
        hc, _ = _head_of_slot(c)
        if row_natural:
            return (r >= hc * DH) & (r < hc * DH + DH)
        hr, _ = _head_of_slot(r)
        return hr == hc

    d_wcatT[...] = jnp.zeros_like(d_wcatT)
    d_wo[...] = jnp.zeros_like(d_wo)
    d_win[...] = jnp.zeros_like(d_win)
    d_wout[...] = jnp.zeros_like(d_wout)
    pmat[...] = perm_matrix()
    in_cp[IN_WPHI].wait()
    in_cp[IN_WQKV].wait()
    mm[...] = jnp.where(head_mask((D, D), True), mm[...], jnp.zeros((), bf16))
    for i in (IN_WIN, IN_WSP, IN_BSP, IN_WOUT, IN_GOUT):
        in_cp[i].start()

    def band_right(lhs_ref, c0, m_ref, out_ref, outT_ref):
        for (b0, b1, a0, a1) in BANDS:
            res = _dot_nn(lhs_ref[:, c0 + 128 * a0:c0 + 128 * a1],
                          m_ref[128 * a0:128 * a1, 128 * b0:128 * b1])
            out_ref[:, c0 + 128 * b0:c0 + 128 * b1] = res.astype(bf16)
            outT_ref[c0 + 128 * b0:c0 + 128 * b1, :] = jnp.transpose(res).astype(bf16)

    band_right(wqkv, 0, mm, wcat, wcatT)
    band_right(wqkv, D, mm, wcat, wcatT)
    band_right(wqkv, 2 * D, pmat, wcat, wcatT)
    in_cp[IN_WO].wait()
    for (b0, b1, a0, a1) in BANDS:
        wop[128 * b0:128 * b1, :] = _dot_tn(
            pmat[128 * a0:128 * a1, 128 * b0:128 * b1], wo[128 * a0:128 * a1, :]).astype(bf16)
    in_cp[IN_X].wait()

    GR = DH * G

    def grp_phi(ph, g):
        return jnp.concatenate(
            [ph[GR * g:GR * (g + 1), :], ph[D + GR * g:D + GR * (g + 1), :]], axis=0)

    def acc_bands(vT, phT):
        for g in range(NG):
            acc[g, 0:GR, 0:2 * GR] += _dot_nt(vT[GR * g:GR * (g + 1), :], grp_phi(phT, g))

    def finish_acc(m_ref, mT_ref):
        r = lax.broadcasted_iota(jnp.int32, (256, 384), 0)
        c = lax.broadcasted_iota(jnp.int32, (256, 384), 1)
        same = ((r & (G - 1)) == (c & (G - 1))) & (r < GR) & (c < 2 * GR)
        for g in range(NG):
            m = jnp.where(same, acc[g], 0.0)
            m_ref[g] = m.astype(bf16)
            mT_ref[g] = jnp.transpose(m).astype(bf16)

    def apply_to_v(m_ref, phT):
        outs = []
        for g in range(NG):
            outs.append(_dot_nn(m_ref[g, 0:GR, 0:2 * GR], grp_phi(phT, g)))
        return jnp.concatenate(outs, axis=0)

    def apply_to_phi(mT_ref, vT):
        plus, minus = [], []
        for g in range(NG):
            res = _dot_nn(mT_ref[g, 0:2 * GR, 0:GR], vT[GR * g:GR * (g + 1), :])
            plus.append(res[:GR, :])
            minus.append(res[GR:, :])
        return jnp.concatenate(plus, axis=0), jnp.concatenate(minus, axis=0)

    def fold_col(ref):
        ref[...] = jnp.broadcast_to(jnp.sum(ref[...], axis=1, keepdims=True), ref.shape)

    def inv_den(phq_f, slot):
        pz = phq_f * _lane_tile(zcol[slot])
        den = (jnp.sum(_to4(pz[0:D]), axis=1, keepdims=True)
               + jnp.sum(_to4(pz[D:2 * D]), axis=1, keepdims=True))
        return 1.0 / (den + DEN_EPS)

    def a_fwd(layer):
        first = layer == 0
        slot = layer // 2
        acc[...] = jnp.zeros_like(acc)
        zcol[slot] = jnp.zeros((2 * D, 128), f32)

        def get_x(rows):
            return x_in[rows, :].astype(f32) if first else xres[rows, :]

        def ln_in(rows):
            xn, rstd = _ln_fwd(get_x(rows))
            stats[rows, layer:layer + 1] = rstd
            a_xn[rows, :] = xn.astype(bf16)

        ln_in(pl.ds(0, T))

        def phase1(rows, nrows):
            xnb = a_xn[rows, :]
            pk = _dot_nt(wcatT[D:2 * D, :], xnb)
            ln_in(nrows)
            vb = _dot_nt(wcatT[2 * D:3 * D, :], xnb).astype(bf16)
            a_v[:, rows] = vb
            kp, km = _softmax_pm(pk)
            pq = _dot_nt(wcatT[0:D, :], xnb)
            phik = jnp.concatenate([_from4(kp), _from4(km)], axis=0).astype(bf16)
            a_pk[:, rows] = phik
            acc_bands(vb, phik)
            qp, qm = _softmax_pm(pq)
            a_pq[0:D, rows] = _from4(qp).astype(bf16)
            a_pq[D:2 * D, rows] = _from4(qm).astype(bf16)
            zcol[slot] += _lane_fold(phik.astype(f32))

        row_loop_pf(phase1, "a_fwd_p1")
        finish_acc(kvm.at[slot], kvT.at[slot])
        fold_col(zcol.at[slot])

        def phase2(rows):
            phq = a_pq[:, rows]
            num = apply_to_v(kvm.at[slot], phq)
            inv = inv_den(phq.astype(f32), slot)
            o = _from4(_to4(num) * inv).astype(bf16)
            a_o[:, rows] = o
            xres[rows, :] = get_x(rows) + _dot_tn(o, wop[...])

        row_loop(phase2, "a_fwd_p2")

    def b_fwd(layer):
        slot = layer // 2
        last = layer == 3

        def ln_in(rows):
            xn, rstd = _ln_fwd(xres[rows, :])
            stats[rows, layer:layer + 1] = rstd
            b_xn[rows, :] = xn.astype(bf16)

        ln_in(pl.ds(0, T))

        def phase1(rows, nrows):
            xnb = b_xn[rows, :]

            def gelu_chunk(u, c0):
                u2 = u * u
                th = jnp.tanh(u * ((GELU_C * GELU_A) * u2 + GELU_C))
                hp = 0.5 * th + 0.5
                zz = u * hp
                gp = hp + (zz * (1.0 - hp)) * ((6.0 * GELU_C * GELU_A) * u2 + 2.0 * GELU_C)
                b_gp[rows, c0:c0 + u.shape[1]] = gp.astype(bf16)
                return zz

            ub = _dot_nn(xnb, win[:, FH:F])
            ln_in(nrows)
            ua = _dot_nn(xnb, win[:, 0:FH // 2])
            zzb = gelu_chunk(ub, FH)
            zn, rstd2 = _ln_fwd(zzb)
            stats[rows, 4 + slot:5 + slot] = rstd2
            z2[slot, rows, :] = zn.astype(bf16)
            uc = _dot_nn(xnb, win[:, FH // 2:FH])
            b_z1[rows, 0:FH // 2] = gelu_chunk(ua, 0).astype(bf16)
            b_z1[rows, FH // 2:FH] = gelu_chunk(uc, FH // 2).astype(bf16)

        row_loop_pf(phase1, "b_fwd_p1")

        def phase2(rows):
            g = _dot_nn(wsp[rows, :], z2[slot]) + bcol[rows, 0:1]
            b_g[rows, :] = g.astype(bf16)
            y = (b_z1[rows, :].astype(f32) * g).astype(bf16)
            xnew = xres[rows, :] + _dot_nn(y, wout[...])
            if last:
                x_in[rows, :] = xnew.astype(bf16)
            else:
                xres[rows, :] = xnew

        row_loop(phase2, "b_fwd_p2")

    def b_bwd(layer):
        slot = layer // 2
        first = layer == 3

        def get_d(rows):
            return gout[rows, :].astype(f32) if first else xres[rows, :]

        def phase1(rows):
            dob = get_d(rows).astype(bf16)
            dy = _dot_nt(dob, wout[...])
            z1 = b_z1[rows, :].astype(f32)
            g = b_g[rows, :].astype(f32)
            y = (z1 * g).astype(bf16)
            d_wout[...] += _dot_tn(y, dob)
            dgv = dy * z1
            dg[slot, rows, :] = dgv.astype(bf16)
            tmp[rows, :] = (dy * g * b_gp[rows, 0:FH].astype(f32)).astype(bf16)

        row_loop(phase1, "b_bwd_p1")

        def phase2(rows):
            dz2 = _dot_tn(wsp[:, rows], dg[slot])
            du1 = tmp[rows, :]
            xn = b_xn[rows, :]
            dxn1 = _dot_nt(du1, win[:, 0:FH])
            dzz = _ln_bwd(dz2, z2[slot, rows, :].astype(f32), stats[rows, 4 + slot:5 + slot])
            du2 = (dzz * b_gp[rows, FH:F].astype(f32)).astype(bf16)
            d_win[:, 0:FH] += _dot_tn(xn, du1)
            dxn = dxn1 + _dot_nt(du2, win[:, FH:F])
            d_win[:, FH:F] += _dot_tn(xn, du2)
            xres[rows, :] = get_d(rows) + _ln_bwd(dxn, xn.astype(f32), stats[rows, layer:layer + 1])

        row_loop(phase2, "b_bwd_p2")

    def a_bwd(layer):
        slot = layer // 2
        last = layer == 0
        acc[...] = jnp.zeros_like(acc)
        dzcol[...] = jnp.zeros_like(dzcol)

        def phase1(rows):
            dob = xres[rows, :].astype(bf16)
            doT = _to4(_dot_nt(wop[...], dob))
            ob = a_o[:, rows]
            d_wo[...] += _dot_nn(ob, dob)
            phq = a_pq[:, rows]
            phqf = phq.astype(f32)
            inv = inv_den(phqf, slot)
            dnum = _from4(doT * inv).astype(bf16)
            dden = -jnp.sum(doT * _to4(ob.astype(f32)), axis=1, keepdims=True) * inv
            dp_p, dp_m = apply_to_phi(kvT.at[slot], dnum)
            acc_bands(dnum, phq)
            zt = _lane_tile(zcol[slot])
            dp_p = _to4(dp_p) + dden * _to4(zt[0:D])
            dp_m = _to4(dp_m) + dden * _to4(zt[D:2 * D])
            pp = _to4(phqf[0:D])
            pmn = _to4(phqf[D:2 * D])
            dzcol[0:D, :] += _lane_fold(_from4(pp * dden))
            dzcol[D:2 * D, :] += _lane_fold(_from4(pmn * dden))
            tmpT[:, rows] = _from4(_softmax_bwd(pp, pmn, dp_p, dp_m)).astype(bf16)

        row_loop(phase1, "a_bwd_p1")
        finish_acc(dkvm, dkvT)
        fold_col(dzcol)

        def phase2(rows):
            vb = a_v[:, rows]
            phk = a_pk[:, rows]
            dp_p, dp_m = apply_to_phi(dkvT, vb)
            dv = apply_to_v(dkvm, phk)
            dzt = _lane_tile(dzcol[...])
            dp_p = _to4(dp_p + dzt[0:D])
            dp_m = _to4(dp_m + dzt[D:2 * D])
            phkf = phk.astype(f32)
            dpk = _softmax_bwd(_to4(phkf[0:D]), _to4(phkf[D:2 * D]), dp_p, dp_m)
            dPT = jnp.concatenate(
                [tmpT[:, rows], _from4(dpk).astype(bf16), dv.astype(bf16)], axis=0)
            dxn = jnp.transpose(_dot_nn(wcat[...], dPT))
            xn = a_xn[rows, :]
            d_wcatT[...] += _dot_nn(dPT, xn)
            dxnew = xres[rows, :] + _ln_bwd(dxn, xn.astype(f32), stats[rows, layer:layer + 1])
            if last:
                gout[rows, :] = dxnew.astype(bf16)
            else:
                xres[rows, :] = dxnew

        row_loop(phase2, "a_bwd_p2")

    def out_copy(i, src, dst):
        return pltpu.make_async_copy(src, dst, out_sems.at[i])

    a_fwd(0)
    spA_out = spill(setA, 0, True)
    start_all(spA_out)

    in_cp[IN_WIN].wait()
    in_cp[IN_WSP].wait()
    in_cp[IN_BSP].wait()
    in_cp[IN_WOUT].wait()
    bcol[...] = jnp.transpose(jnp.broadcast_to(bsp[...].astype(f32), (128, S)))
    b_fwd(1)
    spB_out = spill(setB, 5, True)
    start_all(spB_out)

    wait_all(spA_out)
    a_fwd(2)
    wait_all(spB_out)
    b_fwd(3)
    cp_out = out_copy(0, x_in, out_hbm)
    cp_out.start()

    in_cp[IN_GOUT].wait()
    b_bwd(3)
    spB_in = spill(setB, 5, False)
    start_all(spB_in)
    a_bwd(2)
    spA_in = spill(setA, 0, False)
    start_all(spA_in)
    wait_all(spB_in)
    b_bwd(1)

    win[...] = d_win[...].astype(bf16)
    cp_gwin = out_copy(5, win, gwin_hbm)
    cp_gwin.start()
    wout[...] = d_wout[...].astype(bf16)
    cp_gwout = out_copy(8, wout, gwout_hbm)
    cp_gwout.start()

    def wsp_grad(rows):
        wsp[rows, :] = (_dot_nt(dg[0, rows, :], z2[0]) + _dot_nt(dg[1, rows, :], z2[1])).astype(bf16)
        bcol[rows, :] = jnp.broadcast_to(
            jnp.sum(dg[0, rows, :].astype(f32) + dg[1, rows, :].astype(f32), axis=1, keepdims=True),
            (T, 128))

    row_loop(wsp_grad, "wsp_grad")
    cp_gwsp = out_copy(6, wsp, gwsp_hbm)
    cp_gwsp.start()
    gb_st[...] = jnp.transpose(bcol[...])[0:1, :].astype(bf16)
    cp_gb = out_copy(7, gb_st, gbsp_hbm)
    cp_gb.start()

    wait_all(spA_in)
    a_bwd(0)
    cp_gx = out_copy(1, gout, gx_hbm)
    cp_gx.start()

    wcatT[...] = d_wcatT[...].astype(bf16)
    rr = lax.broadcasted_iota(jnp.int32, (D, 128), 0)
    rc = lax.broadcasted_iota(jnp.int32, (D, 128), 1)
    rmat = (_d_of_slot(rr) == rc).astype(bf16)
    hm = head_mask((D, D), True)
    for (a0, a1, b0, b1) in BANDS:
        dMT = (_dot_nn(wcatT[128 * b0:128 * b1, :], wqkv[:, 128 * a0:128 * a1])
               + _dot_nn(wcatT[D + 128 * b0:D + 128 * b1, :], wqkv[:, D + 128 * a0:D + 128 * a1]))
        dM = jnp.where(hm[128 * a0:128 * a1, 128 * b0:128 * b1], jnp.transpose(dMT), 0.0)
        res = _dot_nn(dM.astype(bf16), rmat[128 * b0:128 * b1, :])
        gphi_st[128 * a0:128 * a1, :] = res[:, 0:DH].astype(bf16)
    cp_gphi = out_copy(3, gphi_st, gwphi_hbm)
    cp_gphi.start()

    for c0, m_ref in ((0, mm), (D, mm), (2 * D, pmat)):
        for (a0, a1, b0, b1) in BANDS:
            res = _dot_nn(m_ref[128 * a0:128 * a1, 128 * b0:128 * b1],
                          wcatT[c0 + 128 * b0:c0 + 128 * b1, :])
            wcat[:, c0 + 128 * a0:c0 + 128 * a1] = jnp.transpose(res).astype(bf16)
    cp_gwqkv = out_copy(2, wcat, gwqkv_hbm)
    cp_gwqkv.start()
    for (a0, a1, b0, b1) in BANDS:
        wo[128 * a0:128 * a1, :] = _dot_nn(
            pmat[128 * a0:128 * a1, 128 * b0:128 * b1],
            d_wo[128 * b0:128 * b1, :].astype(bf16)).astype(bf16)
    cp_gwo = out_copy(4, wo, gwo_hbm)
    cp_gwo.start()
    for c in (cp_out, cp_gwin, cp_gwout, cp_gwsp, cp_gb, cp_gx, cp_gphi, cp_gwqkv, cp_gwo):
        c.wait()


@jax.jit
def pallas_interleave_layers__linear_kernel_hedgehog__mixer_gmlp__prompt_kernel(
    A_x: jax.Array,
    A_wqkv: jax.Array,
    A_w_phi: jax.Array,
    A_wo: jax.Array,
    B_x: jax.Array,
    B_w_in: jax.Array,
    B_w_sp: jax.Array,
    B_b_sp: jax.Array,
    B_w_out: jax.Array,
    grad_out: jax.Array,
):
    del B_x
    x2 = A_x.reshape(S, D)
    g2 = grad_out.reshape(S, D)
    wphi_b = jnp.broadcast_to(
        A_w_phi.reshape(H * DH, 1, DH, 1), (H * DH, NG, DH, G)).reshape(D, D)
    bsp2 = B_b_sp.reshape(1, S)

    sds = jax.ShapeDtypeStruct
    out_shape = (
        sds((S, D), bf16),
        sds((S, D), bf16),
        sds((D, 3 * D), bf16),
        sds((H * DH, DH), bf16),
        sds((D, D), bf16),
        sds((D, F), bf16),
        sds((S, S), bf16),
        sds((1, S), bf16),
        sds((FH, D), bf16),
        sds((S, D), bf16), sds((2 * D, S), bf16), sds((2 * D, S), bf16),
        sds((D, S), bf16), sds((D, S), bf16),
        sds((S, D), bf16), sds((S, FH), bf16), sds((S, F), bf16), sds((S, FH), bf16),
    )
    any_spec = pl.BlockSpec(memory_space=pl.ANY)
    V = pltpu.VMEM
    scratch = [
        V((S, D), bf16),
        V((S, D), bf16),
        V((D, 3 * D), bf16),
        V((D, D), bf16),
        V((D, D), bf16),
        V((D, F), bf16),
        V((S, S), bf16),
        V((1, S), bf16),
        V((FH, D), bf16),
        V((D, 3 * D), bf16),
        V((3 * D, D), bf16),
        V((D, D), bf16),
        V((S, D), f32),
        V((S, D), bf16),
        V((2 * D, S), bf16),
        V((2 * D, S), bf16),
        V((D, S), bf16),
        V((D, S), bf16),
        V((S, D), bf16),
        V((S, FH), bf16),
        V((S, F), bf16),
        V((S, FH), bf16),
        V((2, S, FH), bf16),
        V((2, S, FH), bf16),
        V((S, FH), bf16),
        V((D, S), bf16),
        V((2, NG, 256, 384), bf16),
        V((2, NG, 384, 256), bf16),
        V((2, 2 * D, 128), f32),
        V((NG, 256, 384), f32),
        V((NG, 256, 384), bf16),
        V((NG, 384, 256), bf16),
        V((2 * D, 128), f32),
        V((D, D), bf16),
        V((3 * D, D), f32),
        V((D, D), f32),
        V((D, F), f32),
        V((FH, D), f32),
        V((S, 128), f32),
        V((S, 128), f32),
        V((D, DH), bf16),
        V((1, S), bf16),
        pltpu.SemaphoreType.DMA((9,)),
        pltpu.SemaphoreType.DMA((9,)),
        pltpu.SemaphoreType.DMA((9,)),
    ]
    outs = pl.pallas_call(
        _kernel,
        out_shape=out_shape,
        in_specs=[any_spec] * 9,
        out_specs=tuple([any_spec] * len(out_shape)),
        scratch_shapes=scratch,
        compiler_params=pltpu.CompilerParams(vmem_limit_bytes=124 * 1024 * 1024),
    )(x2, A_wqkv, wphi_b, A_wo, B_w_in, B_w_sp, bsp2, B_w_out, g2)

    return (
        outs[0].reshape(1, S, D),
        outs[1].reshape(1, S, D),
        outs[2],
        outs[3].reshape(H, DH, DH),
        outs[4],
        outs[5],
        outs[6],
        outs[7].reshape(S),
        outs[8],
    )
```

```python
import jax
import jax.numpy as jnp
from jax import lax
import jax.experimental.pallas as pl
import jax.experimental.pallas.tpu as pltpu

S, D, H, DH = 2048, 640, 32, 20
F, FH = 1536, 768
NTL = D // 128
G = 8
NG = H // G
T = 512
NR = S // T
LN_EPS = 1e-5
DEN_EPS = 1e-6
GELU_C = 0.7978845608028654
GELU_A = 0.044715

f32 = jnp.float32
bf16 = jnp.bfloat16


def _dot_nn(a, b):
    return lax.dot_general(a, b, (((1,), (0,)), ((), ())), preferred_element_type=f32)


def _dot_nt(a, b):
    return lax.dot_general(a, b, (((1,), (1,)), ((), ())), preferred_element_type=f32)


def _dot_tn(a, b):
    return lax.dot_general(a, b, (((0,), (0,)), ((), ())), preferred_element_type=f32)


def _tile_groups(j):
    return [g for g in range(NG)
            if DH * G * g < 128 * (j + 1) and DH * G * (g + 1) > 128 * j]


def _bands():
    bands = []
    for a in range(NTL):
        ga = set(_tile_groups(a))
        bs = [b for b in range(NTL) if ga & set(_tile_groups(b))]
        rng = (min(bs), max(bs) + 1)
        if bands and tuple(bands[-1][2:]) == rng:
            bands[-1][1] = a + 1
        else:
            bands.append([a, a + 1, rng[0], rng[1]])
    return [tuple(b) for b in bands]


BANDS = _bands()


def _head_of_slot(c):
    grp = jnp.zeros_like(c)
    for g in range(1, NG):
        grp = grp + (c >= DH * G * g).astype(jnp.int32)
    return grp * G + (c & (G - 1)), grp


def _d_of_slot(c):
    _, grp = _head_of_slot(c)
    return lax.shift_right_logical(c - grp * (DH * G), jnp.int32(G.bit_length() - 1))


def _to4(a):
    return a.reshape(NG, DH, G, a.shape[-1])


def _from4(a):
    return a.reshape(D, a.shape[-1])


def _softmax_pm(p):
    p4 = _to4(p)
    mx = jnp.max(p4, axis=1, keepdims=True)
    mn = jnp.min(p4, axis=1, keepdims=True)
    ep = jnp.exp(p4 - mx)
    en = jnp.exp(mn - p4)
    ip = 1.0 / jnp.sum(ep, axis=1, keepdims=True)
    im = 1.0 / jnp.sum(en, axis=1, keepdims=True)
    return ep * ip, en * im


def _softmax_bwd(pp, pmn, dpp, dpm):
    ap = pp * dpp
    am = pmn * dpm
    sp = jnp.sum(ap, axis=1, keepdims=True)
    sm = jnp.sum(am, axis=1, keepdims=True)
    return (ap - pp * sp) - (am - pmn * sm)


def _ln_fwd(x):
    mu = jnp.mean(x, axis=1, keepdims=True)
    xc = x - mu
    var = jnp.mean(xc * xc, axis=1, keepdims=True)
    rstd = lax.rsqrt(var + LN_EPS)
    return xc * rstd, rstd


def _ln_bwd(dy, y, rstd):
    m1 = jnp.mean(dy, axis=1, keepdims=True)
    m2 = jnp.mean(dy * y, axis=1, keepdims=True)
    return rstd * (dy - m1 - y * m2)


def _lane_tile(col):
    return jnp.concatenate([col] * (T // 128), axis=1)


def _lane_fold(a):
    out = a[:, 0:128]
    for j in range(1, T // 128):
        out = out + a[:, 128 * j:128 * (j + 1)]
    return out


def _kernel(
    x_hbm, wqkv_hbm, wphi_hbm, wo_hbm, win_hbm, wsp_hbm, bsp_hbm, wout_hbm, gout_hbm,
    out_hbm, gx_hbm, gwqkv_hbm, gwphi_hbm, gwo_hbm, gwin_hbm, gwsp_hbm, gbsp_hbm, gwout_hbm,
    sA_xn, sA_pq, sA_pk, sA_v, sA_o, sB_xn, sB_z1, sB_gp, sB_g,
    x_in, gout, wqkv, mm, wo, win, wsp, bsp, wout, wcat, wcatT, wop,
    xres, a_xn, a_pq, a_pk, a_v, a_o, b_xn, b_z1, b_gp, b_g,
    z2, dg, tmp, tmpT, kvm, kvT, zcol, acc, dkvm, dkvT, dzcol, pmat,
    d_wcatT, d_wo, d_win, d_wout, stats, bcol, gphi_st, gb_st,
    in_sems, out_sems, sp_sems,
):
    in_pairs = [(x_hbm, x_in), (wqkv_hbm, wqkv), (wphi_hbm, mm), (wo_hbm, wo),
                (win_hbm, win), (wsp_hbm, wsp), (bsp_hbm, bsp), (wout_hbm, wout),
                (gout_hbm, gout)]
    in_cp = [pltpu.make_async_copy(s, d, in_sems.at[i]) for i, (s, d) in enumerate(in_pairs)]
    (IN_X, IN_WQKV, IN_WPHI, IN_WO, IN_WIN, IN_WSP, IN_BSP, IN_WOUT, IN_GOUT) = range(9)
    for i in (IN_WPHI, IN_WQKV, IN_X, IN_WO):
        in_cp[i].start()

    setA = [(a_xn, sA_xn), (a_pq, sA_pq), (a_pk, sA_pk), (a_v, sA_v), (a_o, sA_o)]
    setB = [(b_xn, sB_xn), (b_z1, sB_z1), (b_gp, sB_gp), (b_g, sB_g)]

    def spill(bufs, base, to_hbm):
        cps = []
        for i, (v, h) in enumerate(bufs):
            src, dst = (v, h) if to_hbm else (h, v)
            cps.append(pltpu.make_async_copy(src, dst, sp_sems.at[base + i]))
        return cps

    def start_all(cps):
        for c in cps:
            c.start()

    def wait_all(cps):
        for c in cps:
            c.wait()

    def row_loop(body, name):
        del name

        def wrapped(i, c):
            body(pl.ds(pl.multiple_of(i * T, T), T))
            return c
        lax.fori_loop(0, NR, wrapped, 0)

    def row_loop_pf(body, name):
        del name

        def wrapped(i, c):
            nxt = jnp.minimum(i + 1, NR - 1)
            body(pl.ds(pl.multiple_of(i * T, T), T), pl.ds(pl.multiple_of(nxt * T, T), T))
            return c
        lax.fori_loop(0, NR, wrapped, 0)

    def perm_matrix():
        r = lax.broadcasted_iota(jnp.int32, (D, D), 0)
        c = lax.broadcasted_iota(jnp.int32, (D, D), 1)
        hc, _ = _head_of_slot(c)
        return (r == hc * DH + _d_of_slot(c)).astype(bf16)

    def head_mask(shape, row_natural):
        r = lax.broadcasted_iota(jnp.int32, shape, 0)
        c = lax.broadcasted_iota(jnp.int32, shape, 1)
        if shape[1] > D:
            c = jnp.where(c >= D, c - D, c)
        hc, _ = _head_of_slot(c)
        if row_natural:
            return (r >= hc * DH) & (r < hc * DH + DH)
        hr, _ = _head_of_slot(r)
        return hr == hc

    d_wcatT[...] = jnp.zeros_like(d_wcatT)
    d_wo[...] = jnp.zeros_like(d_wo)
    d_win[...] = jnp.zeros_like(d_win)
    d_wout[...] = jnp.zeros_like(d_wout)
    pmat[...] = perm_matrix()
    in_cp[IN_WPHI].wait()
    in_cp[IN_WQKV].wait()
    mm[...] = jnp.where(head_mask((D, D), True), mm[...], jnp.zeros((), bf16))
    for i in (IN_WIN, IN_WSP, IN_BSP, IN_WOUT, IN_GOUT):
        in_cp[i].start()

    def band_right(lhs_ref, c0, m_ref, out_ref, outT_ref):
        for (b0, b1, a0, a1) in BANDS:
            res = _dot_nn(lhs_ref[:, c0 + 128 * a0:c0 + 128 * a1],
                          m_ref[128 * a0:128 * a1, 128 * b0:128 * b1])
            out_ref[:, c0 + 128 * b0:c0 + 128 * b1] = res.astype(bf16)
            outT_ref[c0 + 128 * b0:c0 + 128 * b1, :] = jnp.transpose(res).astype(bf16)

    band_right(wqkv, 0, mm, wcat, wcatT)
    band_right(wqkv, D, mm, wcat, wcatT)
    band_right(wqkv, 2 * D, pmat, wcat, wcatT)
    in_cp[IN_WO].wait()
    for (b0, b1, a0, a1) in BANDS:
        wop[128 * b0:128 * b1, :] = _dot_tn(
            pmat[128 * a0:128 * a1, 128 * b0:128 * b1], wo[128 * a0:128 * a1, :]).astype(bf16)
    in_cp[IN_X].wait()

    GR = DH * G

    def grp_phi(ph, g):
        return jnp.concatenate(
            [ph[GR * g:GR * (g + 1), :], ph[D + GR * g:D + GR * (g + 1), :]], axis=0)

    def acc_bands(vT, phT):
        for g in range(NG):
            acc[g, 0:GR, 0:2 * GR] += _dot_nt(vT[GR * g:GR * (g + 1), :], grp_phi(phT, g))

    def finish_acc(m_ref, mT_ref):
        r = lax.broadcasted_iota(jnp.int32, (256, 384), 0)
        c = lax.broadcasted_iota(jnp.int32, (256, 384), 1)
        same = ((r & (G - 1)) == (c & (G - 1))) & (r < GR) & (c < 2 * GR)
        for g in range(NG):
            m = jnp.where(same, acc[g], 0.0)
            m_ref[g] = m.astype(bf16)
            mT_ref[g] = jnp.transpose(m).astype(bf16)

    def apply_to_v(m_ref, phT):
        outs = []
        for g in range(NG):
            outs.append(_dot_nn(m_ref[g, 0:GR, 0:2 * GR], grp_phi(phT, g)))
        return jnp.concatenate(outs, axis=0)

    def apply_to_phi(mT_ref, vT):
        plus, minus = [], []
        for g in range(NG):
            res = _dot_nn(mT_ref[g, 0:2 * GR, 0:GR], vT[GR * g:GR * (g + 1), :])
            plus.append(res[:GR, :])
            minus.append(res[GR:, :])
        return jnp.concatenate(plus, axis=0), jnp.concatenate(minus, axis=0)

    def fold_col(ref):
        ref[...] = jnp.broadcast_to(jnp.sum(ref[...], axis=1, keepdims=True), ref.shape)

    def inv_den(phq_f, slot):
        pz = phq_f * _lane_tile(zcol[slot])
        den = (jnp.sum(_to4(pz[0:D]), axis=1, keepdims=True)
               + jnp.sum(_to4(pz[D:2 * D]), axis=1, keepdims=True))
        return 1.0 / (den + DEN_EPS)

    def a_fwd(layer):
        first = layer == 0
        slot = layer // 2
        acc[...] = jnp.zeros_like(acc)
        zcol[slot] = jnp.zeros((2 * D, 128), f32)

        def get_x(rows):
            return x_in[rows, :].astype(f32) if first else xres[rows, :]

        def ln_in(rows):
            xn, rstd = _ln_fwd(get_x(rows))
            stats[rows, layer:layer + 1] = rstd
            a_xn[rows, :] = xn.astype(bf16)

        ln_in(pl.ds(0, T))

        def phase1(rows, nrows):
            xnb = a_xn[rows, :]
            pk = _dot_nt(wcatT[D:2 * D, :], xnb)
            ln_in(nrows)
            vb = _dot_nt(wcatT[2 * D:3 * D, :], xnb).astype(bf16)
            a_v[:, rows] = vb
            kp, km = _softmax_pm(pk)
            pq = _dot_nt(wcatT[0:D, :], xnb)
            phik = jnp.concatenate([_from4(kp), _from4(km)], axis=0).astype(bf16)
            a_pk[:, rows] = phik
            acc_bands(vb, phik)
            qp, qm = _softmax_pm(pq)
            a_pq[0:D, rows] = _from4(qp).astype(bf16)
            a_pq[D:2 * D, rows] = _from4(qm).astype(bf16)
            zcol[slot] += _lane_fold(phik.astype(f32))

        row_loop_pf(phase1, "a_fwd_p1")
        finish_acc(kvm.at[slot], kvT.at[slot])
        fold_col(zcol.at[slot])

        def phase2(rows):
            phq = a_pq[:, rows]
            num = apply_to_v(kvm.at[slot], phq)
            inv = inv_den(phq.astype(f32), slot)
            o = _from4(_to4(num) * inv).astype(bf16)
            a_o[:, rows] = o
            xres[rows, :] = get_x(rows) + _dot_tn(o, wop[...])

        row_loop(phase2, "a_fwd_p2")

    def b_fwd(layer):
        slot = layer // 2
        last = layer == 3

        def ln_in(rows):
            xn, rstd = _ln_fwd(xres[rows, :])
            stats[rows, layer:layer + 1] = rstd
            b_xn[rows, :] = xn.astype(bf16)

        ln_in(pl.ds(0, T))

        def phase1(rows, nrows):
            xnb = b_xn[rows, :]

            def gelu_chunk(u, c0):
                u2 = u * u
                th = jnp.tanh(u * ((GELU_C * GELU_A) * u2 + GELU_C))
                hp = 0.5 * th + 0.5
                zz = u * hp
                gp = hp + (zz * (1.0 - hp)) * ((6.0 * GELU_C * GELU_A) * u2 + 2.0 * GELU_C)
                b_gp[rows, c0:c0 + u.shape[1]] = gp.astype(bf16)
                return zz

            ub = _dot_nn(xnb, win[:, FH:F])
            ln_in(nrows)
            ua = _dot_nn(xnb, win[:, 0:FH // 2])
            zzb = gelu_chunk(ub, FH)
            zn, rstd2 = _ln_fwd(zzb)
            stats[rows, 4 + slot:5 + slot] = rstd2
            z2[slot, rows, :] = zn.astype(bf16)
            uc = _dot_nn(xnb, win[:, FH // 2:FH])
            b_z1[rows, 0:FH // 2] = gelu_chunk(ua, 0).astype(bf16)
            b_z1[rows, FH // 2:FH] = gelu_chunk(uc, FH // 2).astype(bf16)

        row_loop_pf(phase1, "b_fwd_p1")

        def phase2(rows):
            g = _dot_nn(wsp[rows, :], z2[slot]) + bcol[rows, 0:1]
            b_g[rows, :] = g.astype(bf16)
            y = (b_z1[rows, :].astype(f32) * g).astype(bf16)
            xnew = xres[rows, :] + _dot_nn(y, wout[...])
            if last:
                x_in[rows, :] = xnew.astype(bf16)
            else:
                xres[rows, :] = xnew

        row_loop(phase2, "b_fwd_p2")

    def b_bwd(layer):
        slot = layer // 2
        first = layer == 3

        def get_d(rows):
            return gout[rows, :].astype(f32) if first else xres[rows, :]

        def phase1(rows):
            dob = get_d(rows).astype(bf16)
            dy = _dot_nt(dob, wout[...])
            z1 = b_z1[rows, :].astype(f32)
            g = b_g[rows, :].astype(f32)
            y = (z1 * g).astype(bf16)
            d_wout[...] += _dot_tn(y, dob)
            dgv = dy * z1
            dg[slot, rows, :] = dgv.astype(bf16)
            tmp[rows, :] = (dy * g * b_gp[rows, 0:FH].astype(f32)).astype(bf16)

        row_loop(phase1, "b_bwd_p1")

        def phase2(rows):
            dz2 = _dot_tn(wsp[:, rows], dg[slot])
            du1 = tmp[rows, :]
            xn = b_xn[rows, :]
            dxn1 = _dot_nt(du1, win[:, 0:FH])
            dzz = _ln_bwd(dz2, z2[slot, rows, :].astype(f32), stats[rows, 4 + slot:5 + slot])
            du2 = (dzz * b_gp[rows, FH:F].astype(f32)).astype(bf16)
            d_win[:, 0:FH] += _dot_tn(xn, du1)
            dxn = dxn1 + _dot_nt(du2, win[:, FH:F])
            d_win[:, FH:F] += _dot_tn(xn, du2)
            xres[rows, :] = get_d(rows) + _ln_bwd(dxn, xn.astype(f32), stats[rows, layer:layer + 1])

        row_loop(phase2, "b_bwd_p2")

    def a_bwd(layer):
        slot = layer // 2
        last = layer == 0
        acc[...] = jnp.zeros_like(acc)
        dzcol[...] = jnp.zeros_like(dzcol)

        def phase1(rows):
            dob = xres[rows, :].astype(bf16)
            doT = _to4(_dot_nt(wop[...], dob))
            ob = a_o[:, rows]
            d_wo[...] += _dot_nn(ob, dob)
            phq = a_pq[:, rows]
            phqf = phq.astype(f32)
            inv = inv_den(phqf, slot)
            dnum = _from4(doT * inv).astype(bf16)
            dden = -jnp.sum(doT * _to4(ob.astype(f32)), axis=1, keepdims=True) * inv
            dp_p, dp_m = apply_to_phi(kvT.at[slot], dnum)
            acc_bands(dnum, phq)
            zt = _lane_tile(zcol[slot])
            dp_p = _to4(dp_p) + dden * _to4(zt[0:D])
            dp_m = _to4(dp_m) + dden * _to4(zt[D:2 * D])
            pp = _to4(phqf[0:D])
            pmn = _to4(phqf[D:2 * D])
            dzcol[0:D, :] += _lane_fold(_from4(pp * dden))
            dzcol[D:2 * D, :] += _lane_fold(_from4(pmn * dden))
            tmpT[:, rows] = _from4(_softmax_bwd(pp, pmn, dp_p, dp_m)).astype(bf16)

        row_loop(phase1, "a_bwd_p1")
        finish_acc(dkvm, dkvT)
        fold_col(dzcol)
        if last:
            for (a0, a1, b0, b1) in BANDS:
                wo[128 * a0:128 * a1, :] = _dot_nn(
                    pmat[128 * a0:128 * a1, 128 * b0:128 * b1],
                    d_wo[128 * b0:128 * b1, :].astype(bf16)).astype(bf16)
            cp_gwo.start()

        def phase2(rows):
            vb = a_v[:, rows]
            phk = a_pk[:, rows]
            dp_p, dp_m = apply_to_phi(dkvT, vb)
            dv = apply_to_v(dkvm, phk)
            dzt = _lane_tile(dzcol[...])
            dp_p = _to4(dp_p + dzt[0:D])
            dp_m = _to4(dp_m + dzt[D:2 * D])
            phkf = phk.astype(f32)
            dpk = _softmax_bwd(_to4(phkf[0:D]), _to4(phkf[D:2 * D]), dp_p, dp_m)
            dPT = jnp.concatenate(
                [tmpT[:, rows], _from4(dpk).astype(bf16), dv.astype(bf16)], axis=0)
            dxn = jnp.transpose(_dot_nn(wcat[...], dPT))
            xn = a_xn[rows, :]
            d_wcatT[...] += _dot_nn(dPT, xn)
            dxnew = xres[rows, :] + _ln_bwd(dxn, xn.astype(f32), stats[rows, layer:layer + 1])
            if last:
                gout[rows, :] = dxnew.astype(bf16)
            else:
                xres[rows, :] = dxnew

        row_loop(phase2, "a_bwd_p2")

    def out_copy(i, src, dst):
        return pltpu.make_async_copy(src, dst, out_sems.at[i])

    cp_gwo = out_copy(4, wo, gwo_hbm)

    a_fwd(0)
    spA_out = spill(setA, 0, True)
    start_all(spA_out)

    in_cp[IN_WIN].wait()
    in_cp[IN_WSP].wait()
    in_cp[IN_BSP].wait()
    in_cp[IN_WOUT].wait()
    bcol[...] = jnp.transpose(jnp.broadcast_to(bsp[...].astype(f32), (128, S)))
    b_fwd(1)
    spB_out = spill(setB, 5, True)
    start_all(spB_out)

    wait_all(spA_out)
    a_fwd(2)
    wait_all(spB_out)
    b_fwd(3)
    cp_out = out_copy(0, x_in, out_hbm)
    cp_out.start()

    in_cp[IN_GOUT].wait()
    b_bwd(3)
    spB_in = spill(setB, 5, False)
    start_all(spB_in)
    a_bwd(2)
    spA_in = spill(setA, 0, False)
    start_all(spA_in)
    wait_all(spB_in)
    b_bwd(1)

    win[...] = d_win[...].astype(bf16)
    cp_gwin = out_copy(5, win, gwin_hbm)
    cp_gwin.start()
    wout[...] = d_wout[...].astype(bf16)
    cp_gwout = out_copy(8, wout, gwout_hbm)
    cp_gwout.start()

    def wsp_grad(rows):
        wsp[rows, :] = (_dot_nt(dg[0, rows, :], z2[0]) + _dot_nt(dg[1, rows, :], z2[1])).astype(bf16)
        bcol[rows, :] = jnp.broadcast_to(
            jnp.sum(dg[0, rows, :].astype(f32) + dg[1, rows, :].astype(f32), axis=1, keepdims=True),
            (T, 128))

    row_loop(wsp_grad, "wsp_grad")
    cp_gwsp = out_copy(6, wsp, gwsp_hbm)
    cp_gwsp.start()
    gb_st[...] = jnp.transpose(bcol[...])[0:1, :].astype(bf16)
    cp_gb = out_copy(7, gb_st, gbsp_hbm)
    cp_gb.start()

    wait_all(spA_in)
    a_bwd(0)
    cp_gx = out_copy(1, gout, gx_hbm)
    cp_gx.start()

    wcatT[...] = d_wcatT[...].astype(bf16)
    rr = lax.broadcasted_iota(jnp.int32, (D, 128), 0)
    rc = lax.broadcasted_iota(jnp.int32, (D, 128), 1)
    rmat = (_d_of_slot(rr) == rc).astype(bf16)
    hm = head_mask((D, D), True)
    for (a0, a1, b0, b1) in BANDS:
        dMT = (_dot_nn(wcatT[128 * b0:128 * b1, :], wqkv[:, 128 * a0:128 * a1])
               + _dot_nn(wcatT[D + 128 * b0:D + 128 * b1, :], wqkv[:, D + 128 * a0:D + 128 * a1]))
        dM = jnp.where(hm[128 * a0:128 * a1, 128 * b0:128 * b1], jnp.transpose(dMT), 0.0)
        res = _dot_nn(dM.astype(bf16), rmat[128 * b0:128 * b1, :])
        gphi_st[128 * a0:128 * a1, :] = res[:, 0:DH].astype(bf16)
    cp_gphi = out_copy(3, gphi_st, gwphi_hbm)
    cp_gphi.start()

    cp_gwqkv = []
    for c0, m_ref in ((0, mm), (D, mm), (2 * D, pmat)):
        for (a0, a1, b0, b1) in BANDS:
            res = _dot_nn(m_ref[128 * a0:128 * a1, 128 * b0:128 * b1],
                          wcatT[c0 + 128 * b0:c0 + 128 * b1, :])
            wcat[:, c0 + 128 * a0:c0 + 128 * a1] = jnp.transpose(res).astype(bf16)
        cp = pltpu.make_async_copy(wcat.at[:, c0:c0 + D], gwqkv_hbm.at[:, c0:c0 + D],
                                   in_sems.at[c0 // D])
        cp.start()
        cp_gwqkv.append(cp)
    for c in (cp_out, cp_gwin, cp_gwout, cp_gwsp, cp_gb, cp_gx, cp_gphi, cp_gwo, *cp_gwqkv):
        c.wait()


@jax.jit
def pallas_interleave_layers__linear_kernel_hedgehog__mixer_gmlp__prompt_kernel(
    A_x: jax.Array,
    A_wqkv: jax.Array,
    A_w_phi: jax.Array,
    A_wo: jax.Array,
    B_x: jax.Array,
    B_w_in: jax.Array,
    B_w_sp: jax.Array,
    B_b_sp: jax.Array,
    B_w_out: jax.Array,
    grad_out: jax.Array,
):
    del B_x
    x2 = A_x.reshape(S, D)
    g2 = grad_out.reshape(S, D)
    wphi_b = jnp.broadcast_to(
        A_w_phi.reshape(H * DH, 1, DH, 1), (H * DH, NG, DH, G)).reshape(D, D)
    bsp2 = B_b_sp.reshape(1, S)

    sds = jax.ShapeDtypeStruct
    out_shape = (
        sds((S, D), bf16),
        sds((S, D), bf16),
        sds((D, 3 * D), bf16),
        sds((H * DH, DH), bf16),
        sds((D, D), bf16),
        sds((D, F), bf16),
        sds((S, S), bf16),
        sds((1, S), bf16),
        sds((FH, D), bf16),
        sds((S, D), bf16), sds((2 * D, S), bf16), sds((2 * D, S), bf16),
        sds((D, S), bf16), sds((D, S), bf16),
        sds((S, D), bf16), sds((S, FH), bf16), sds((S, F), bf16), sds((S, FH), bf16),
    )
    any_spec = pl.BlockSpec(memory_space=pl.ANY)
    V = pltpu.VMEM
    scratch = [
        V((S, D), bf16),
        V((S, D), bf16),
        V((D, 3 * D), bf16),
        V((D, D), bf16),
        V((D, D), bf16),
        V((D, F), bf16),
        V((S, S), bf16),
        V((1, S), bf16),
        V((FH, D), bf16),
        V((D, 3 * D), bf16),
        V((3 * D, D), bf16),
        V((D, D), bf16),
        V((S, D), f32),
        V((S, D), bf16),
        V((2 * D, S), bf16),
        V((2 * D, S), bf16),
        V((D, S), bf16),
        V((D, S), bf16),
        V((S, D), bf16),
        V((S, FH), bf16),
        V((S, F), bf16),
        V((S, FH), bf16),
        V((2, S, FH), bf16),
        V((2, S, FH), bf16),
        V((S, FH), bf16),
        V((D, S), bf16),
        V((2, NG, 256, 384), bf16),
        V((2, NG, 384, 256), bf16),
        V((2, 2 * D, 128), f32),
        V((NG, 256, 384), f32),
        V((NG, 256, 384), bf16),
        V((NG, 384, 256), bf16),
        V((2 * D, 128), f32),
        V((D, D), bf16),
        V((3 * D, D), f32),
        V((D, D), f32),
        V((D, F), f32),
        V((FH, D), f32),
        V((S, 128), f32),
        V((S, 128), f32),
        V((D, DH), bf16),
        V((1, S), bf16),
        pltpu.SemaphoreType.DMA((9,)),
        pltpu.SemaphoreType.DMA((9,)),
        pltpu.SemaphoreType.DMA((9,)),
    ]
    outs = pl.pallas_call(
        _kernel,
        out_shape=out_shape,
        in_specs=[any_spec] * 9,
        out_specs=tuple([any_spec] * len(out_shape)),
        scratch_shapes=scratch,
        compiler_params=pltpu.CompilerParams(vmem_limit_bytes=124 * 1024 * 1024),
    )(x2, A_wqkv, wphi_b, A_wo, B_w_in, B_w_sp, bsp2, B_w_out, g2)

    return (
        outs[0].reshape(1, S, D),
        outs[1].reshape(1, S, D),
        outs[2],
        outs[3].reshape(H, DH, DH),
        outs[4],
        outs[5],
        outs[6],
        outs[7].reshape(S),
        outs[8],
    )
```
